```python
import jax
import jax.numpy as jnp

def _softmax(x, axis=-1):
    return jax.nn.softmax(x, axis=axis)

def _gelu(x):
    return jax.nn.gelu(x, approximate=True)

def _silu(x):
    return jax.nn.silu(x)

def _sigmoid(x):
    return jax.nn.sigmoid(x)

def _layernorm(x, axis=-1, eps=1e-05):
    m = jnp.mean(x, axis=axis, keepdims=True)
    v = jnp.var(x, axis=axis, keepdims=True)
    return (x - m) / jnp.sqrt(v + eps)

def _scatter_add(tgt, idx, src, axis=0):
    return tgt.at[idx].add(src)

def _segment_sum(src, seg, n):
    return jax.ops.segment_sum(src, seg, n)

class _Rng:

    def __init__(self, key):
        self._k = key

    def _next(self):
        self._k, sub = jax.random.split(self._k)
        return sub

    def normal(self, shape):
        return jax.random.normal(self._next(), shape, dtype=jnp.bfloat16)

    def randint(self, lo, hi, shape):
        return jax.random.randint(self._next(), shape, lo, hi, dtype=jnp.int32)

    def uniform(self, shape, lo=0.0, hi=1.0):
        return jax.random.uniform(self._next(), shape, jnp.bfloat16, lo, hi)

    def permutation(self, n):
        return jax.random.permutation(self._next(), n)
kernel_name = 'adaLN_cond__compressed_kv_cla__dense_activation_relu__decode'

def setup_inputs():
    _rng = _Rng(jax.random.key(int.from_bytes(__import__("os").urandom(4), "little")))
    _w = lambda a: (lambda t: t.astype(jnp.bfloat16) if jnp.issubdtype(t.dtype, jnp.floating) else t)(jnp.asarray(a))

    def _A_setup():
        B, H, Sq, Sk, D, M = (8, 32, 1, 4096, 128, 512)
        Dc = 4 * D
        return {'x': _w((lambda *s: _rng.normal(s) * 0.05)(B, Sq, M)), 'c_kv': _w((lambda *s: _rng.normal(s) * 0.05)(B, Sk, Dc)), 'w_q': _w((lambda *s: _rng.normal(s) * 0.05)(M, H, D) * M ** (-0.5)), 'w_uk': _w((lambda *s: _rng.normal(s) * 0.05)(Dc, H, D) * Dc ** (-0.5)), 'w_uv': _w((lambda *s: _rng.normal(s) * 0.05)(Dc, H, D) * Dc ** (-0.5)), 'w_o': _w((lambda *s: _rng.normal(s) * 0.05)(H, D, M) * (H * D) ** (-0.5))}
    _A_in = _A_setup()

    def _B_setup():
        B, S, D, Dff = (8, 1, 512, 1792)
        return {'x': _w((lambda *s: _rng.normal(s) * 0.05)(B, S, D)), 'w1': _w((lambda *s: _rng.normal(s) * 0.05)(D, Dff)), 'w2': _w((lambda *s: _rng.normal(s) * 0.05)(Dff, D))}
    _B_in = _B_setup()
    return {'A_x': _A_in['x'], 'A_c_kv': _A_in['c_kv'], 'A_w_q': _A_in['w_q'], 'A_w_uk': _A_in['w_uk'], 'A_w_uv': _A_in['w_uv'], 'A_w_o': _A_in['w_o'], 'B_x': _B_in['x'], 'B_w1': _B_in['w1'], 'B_w2': _B_in['w2'], 'c': _w((lambda *s: _rng.normal(s) * 0.05)(8, 512)), 'w_mod': _w((lambda *s: _rng.normal(s) * 0.05)(512, 6 * 512) * 512 ** (-0.5))}

def reference(A_x, A_c_kv, A_w_q, A_w_uk, A_w_uv, A_w_o, B_x, B_w1, B_w2, c, w_mod):

    def _A_ref(x, c_kv, w_q, w_uk, w_uv, w_o):
        B, Sq, M = (x.shape[0], x.shape[1], x.shape[2])
        Sk = c_kv.shape[1]
        H, D = (w_q.shape[1], w_q.shape[2])
        q = jnp.einsum('bqm,mhd->bhqd', x, w_q)
        k = jnp.einsum('bkc,chd->bhkd', c_kv, w_uk)
        v = jnp.einsum('bkc,chd->bhkd', c_kv, w_uv)
        scores = jnp.einsum('bhqd,bhkd->bhqk', q, k) * D ** (-0.5)
        off = Sk - Sq
        qi = jnp.arange(Sq)[:, None]
        kj = jnp.arange(Sk)[None, :]
        cmask = kj <= qi + off
        scores = jnp.where(cmask[None, None], scores, -1000000000.0)
        p = _softmax(scores, axis=-1)
        ctx = jnp.einsum('bhqk,bhkd->bhqd', p, v)
        return jnp.einsum('bhqd,hdm->bqm', ctx, w_o)

    def _B_ref(x, w1, w2):
        h = jnp.einsum('bsd,df->bsf', x, w1)
        zero = jnp.zeros_like(h)
        h = jnp.maximum(h, zero)
        return jnp.einsum('bsf,fd->bsd', h, w2)
    x = A_x
    mod = (_silu(c) @ w_mod).reshape(c.shape[0], 6, 1, -1)
    sa, ca, ga, sb, cb, gb = (mod[:, 0].copy(), mod[:, 1].copy(), mod[:, 2].copy(), mod[:, 3].copy(), mod[:, 4].copy(), mod[:, 5].copy())
    h = _layernorm(x, axis=-1) * (1 + ca) + sa
    x = x + ga * _A_ref(h, A_c_kv, A_w_q, A_w_uk, A_w_uv, A_w_o)
    h = _layernorm(x, axis=-1) * (1 + cb) + sb
    x = x + gb * _B_ref(h, B_w1, B_w2)
    return x
```

```python
import jax
import jax.numpy as jnp
import jax.experimental.pallas as pl
import jax.experimental.pallas.tpu as pltpu

_F32 = jnp.float32
_BF16 = jnp.bfloat16
_NT = (((1,), (1,)), ((), ()))


def _layernorm(x):
    m = jnp.mean(x, axis=-1, keepdims=True)
    d = x - m
    v = jnp.mean(d * d, axis=-1, keepdims=True)
    return d / jnp.sqrt(v + 1e-5)


def _head_pair(w32_ref, j, n, pairs):
    w = w32_ref[pl.ds(j, n, stride=pairs), :]
    lo = pltpu.bitcast(w << 16, _F32).astype(_BF16)
    hi = pltpu.bitcast(w & jnp.uint32(0xFFFF0000), _F32).astype(_BF16)
    return lo, hi


def _build(B, H, Sk, D, M, Dc, F, dma=True, compute=True):
    HP = H // 2
    NC = Dc // 128
    WO_CH = 4
    W2_CH = 7

    def kernel(x_hbm, ckv_hbm, wq_hbm, wuk_hbm, wuv_hbm, wo_hbm, w1_hbm, w2_hbm, c_hbm, wm_hbm,
               o_ref,
               x_v, c_v, ckv_v, wq_v, wuk_v, wuv_v, wo_v, w1_v, w2_v, wma_v, wmb_v,
               qa_v, oc_v, sems, ksems):
        cp = pltpu.make_async_copy
        d_c = cp(c_hbm, c_v, sems.at[0])
        d_wma = cp(wm_hbm.at[:, pl.ds(0, 2 * M)], wma_v, sems.at[1])
        d_x = cp(x_hbm, x_v, sems.at[2])
        d_wq = cp(wq_hbm, wq_v, sems.at[3])
        d_wuk = cp(wuk_hbm, wuk_v, sems.at[4])
        d_kv = lambda b: cp(ckv_hbm.at[b], ckv_v.at[b], ksems.at[b])
        d_wuv = cp(wuv_hbm, wuv_v, sems.at[5])
        d_wmb = cp(wm_hbm.at[:, pl.ds(2 * M, 4 * M)], wmb_v, sems.at[6])
        r = H * D // WO_CH
        d_wo = [cp(wo_hbm.at[pl.ds(i * r, r)], wo_v.at[pl.ds(i * r, r)], sems.at[7 + i]) for i in range(WO_CH)]
        d_w1 = cp(w1_hbm, w1_v, sems.at[7 + WO_CH])
        r2 = F // W2_CH
        d_w2 = [cp(w2_hbm.at[pl.ds(i * r2, r2)], w2_v.at[pl.ds(i * r2, r2)], sems.at[8 + WO_CH + i]) for i in range(W2_CH)]
        start = (lambda d: d.start()) if dma else (lambda d: None)
        wait = (lambda d: d.wait()) if dma else (lambda d: None)

        for d in [d_wma, d_c, d_x, d_wq, d_wuk] + [d_kv(b) for b in range(B)] + [d_wuv, d_wmb] + d_wo + [d_w1] + d_w2:
            start(d)

        wait(d_c)
        cc = c_v[...].astype(_F32)
        sc = (cc * jax.nn.sigmoid(cc)).astype(_BF16)
        wait(d_wma)
        moda = jnp.dot(sc, wma_v[...], preferred_element_type=_F32)
        wait(d_x)
        x = x_v[...].astype(_F32)
        h = (_layernorm(x) * (1.0 + moda[:, M:2 * M]) + moda[:, :M]).astype(_BF16)

        wait(d_wq)
        wq32 = wq_v.bitcast(jnp.uint32)
        qs = []
        for j in range(HP):
            for w in _head_pair(wq32, j, M, HP):
                q = jnp.dot(h, w, preferred_element_type=_F32)
                qs.append((q * D ** -0.5).astype(_BF16))
        wait(d_wuk)
        wuk32 = wuk_v.bitcast(jnp.uint32)
        for j in range(HP):
            for s, w in enumerate(_head_pair(wuk32, j, Dc, HP)):
                hh = 2 * j + s
                qa = jax.lax.dot_general(qs[hh], w, _NT, preferred_element_type=_F32)
                for n in range(NC):
                    qa_v[n, pl.ds(hh, B, stride=H), :] = qa[:, n * 128:(n + 1) * 128]

        def body(b, carry):
            wait(d_kv(b))
            row = pl.ds(pl.multiple_of(b * H, H), H)
            qa = jnp.concatenate([qa_v[n, row, :] for n in range(NC)], axis=1).astype(_BF16)
            s = jax.lax.dot_general(qa, ckv_v[b], _NT, preferred_element_type=_F32)
            m = jnp.max(s, axis=-1, keepdims=True)
            p = jnp.exp(s - m)
            l = jnp.sum(p, axis=-1, keepdims=True)
            o = jnp.dot(p.astype(_BF16), ckv_v[b], preferred_element_type=_F32) / l
            for n in range(NC):
                oc_v[n, row, :] = o[:, n * 128:(n + 1) * 128]
            return carry

        jax.lax.fori_loop(0, B, body, 0)

        wait(d_wuv)
        wuv32 = wuv_v.bitcast(jnp.uint32)
        ctx = []
        for j in range(HP):
            for s, w in enumerate(_head_pair(wuv32, j, Dc, HP)):
                hh = 2 * j + s
                oc = jnp.concatenate([oc_v[n, pl.ds(hh, B, stride=H), :] for n in range(NC)], axis=1)
                ctx.append(jnp.dot(oc.astype(_BF16), w, preferred_element_type=_F32).astype(_BF16))
        wait(d_wmb)
        modb = jnp.dot(sc, wmb_v[...], preferred_element_type=_F32)
        att = None
        hc = H // WO_CH
        for i in range(WO_CH):
            wait(d_wo[i])
            t = jnp.dot(jnp.concatenate(ctx[i * hc:(i + 1) * hc], axis=1), wo_v[pl.ds(i * r, r), :],
                        preferred_element_type=_F32)
            att = t if att is None else att + t
        x1 = x + modb[:, :M] * att
        h2 = (_layernorm(x1) * (1.0 + modb[:, 2 * M:3 * M]) + modb[:, M:2 * M]).astype(_BF16)

        wait(d_w1)
        a = jnp.maximum(jnp.dot(h2, w1_v[...], preferred_element_type=_F32), 0.0).astype(_BF16)
        y = None
        for i in range(W2_CH):
            wait(d_w2[i])
            t = jnp.dot(a[:, i * r2:(i + 1) * r2], w2_v[pl.ds(i * r2, r2), :], preferred_element_type=_F32)
            y = t if y is None else y + t
        o_ref[...] = (x1 + modb[:, 3 * M:] * y).astype(o_ref.dtype)

    scratch = [
        pltpu.VMEM((B, M), _BF16), pltpu.VMEM((B, M), _BF16),
        pltpu.VMEM((B, Sk, Dc), _BF16),
        pltpu.VMEM((M * H, D), _BF16), pltpu.VMEM((Dc * H, D), _BF16), pltpu.VMEM((Dc * H, D), _BF16),
        pltpu.VMEM((H * D, M), _BF16), pltpu.VMEM((M, F), _BF16), pltpu.VMEM((F, M), _BF16),
        pltpu.VMEM((M, 2 * M), _BF16), pltpu.VMEM((M, 4 * M), _BF16),
        pltpu.VMEM((NC, B * H, 128), _F32), pltpu.VMEM((NC, B * H, 128), _F32),
        pltpu.SemaphoreType.DMA((8 + WO_CH + W2_CH,)), pltpu.SemaphoreType.DMA((B,)),
    ]
    return kernel, scratch


def _run(A_x, A_c_kv, A_w_q, A_w_uk, A_w_uv, A_w_o, B_w1, B_w2, c, w_mod, **kw):
    B, Sq, M = A_x.shape
    _, Sk, Dc = A_c_kv.shape
    _, H, D = A_w_q.shape
    F = B_w1.shape[1]
    kernel, scratch = _build(B, H, Sk, D, M, Dc, F, **kw)
    out = pl.pallas_call(
        kernel,
        out_shape=jax.ShapeDtypeStruct((B, M), A_x.dtype),
        in_specs=[pl.BlockSpec(memory_space=pl.ANY)] * 10,
        scratch_shapes=scratch,
        compiler_params=pltpu.CompilerParams(vmem_limit_bytes=100 * 1024 * 1024),
    )(A_x.reshape(B, M), A_c_kv, A_w_q.reshape(M * H, D), A_w_uk.reshape(Dc * H, D),
      A_w_uv.reshape(Dc * H, D), A_w_o.reshape(H * D, M), B_w1, B_w2, c, w_mod)
    return out.reshape(B, Sq, M)


@jax.jit
def pallas_adaLN_cond__compressed_kv_cla__dense_activation_relu__decode_kernel(
    A_x: jax.Array,
    A_c_kv: jax.Array,
    A_w_q: jax.Array,
    A_w_uk: jax.Array,
    A_w_uv: jax.Array,
    A_w_o: jax.Array,
    B_x: jax.Array,
    B_w1: jax.Array,
    B_w2: jax.Array,
    c: jax.Array,
    w_mod: jax.Array,
):
    return _run(A_x, A_c_kv, A_w_q, A_w_uk, A_w_uv, A_w_o, B_w1, B_w2, c, w_mod)
```

```python
import jax
import jax.numpy as jnp
import jax.experimental.pallas as pl
import jax.experimental.pallas.tpu as pltpu

_F32 = jnp.float32
_BF16 = jnp.bfloat16
_NT = (((1,), (1,)), ((), ()))


def _layernorm(x):
    m = jnp.mean(x, axis=-1, keepdims=True)
    d = x - m
    v = jnp.mean(d * d, axis=-1, keepdims=True)
    return d / jnp.sqrt(v + 1e-5)


def _head_pair(w32_ref, j, n, pairs):
    w = w32_ref[pl.ds(j, n, stride=pairs), :]
    lo = pltpu.bitcast(w << 16, _F32).astype(_BF16)
    hi = pltpu.bitcast(w & jnp.uint32(0xFFFF0000), _F32).astype(_BF16)
    return lo, hi


def _build(B, H, Sk, D, M, Dc, F, dma=True, WO_CH=4, W2_CH=7):
    HP = H // 2
    NC = Dc // 128

    def kernel(x_hbm, ckv_hbm, wq_hbm, wuk_hbm, wuv_hbm, wo_hbm, w1_hbm, w2_hbm, c_hbm, wm_hbm,
               o_ref,
               x_v, c_v, ckv_v, wq_v, wuk_v, wuv_v, wo_v, w1_v, w2_v, wma_v, wmb_v,
               qa_v, oc_v, sems, ksems):
        cp = pltpu.make_async_copy
        d_c = cp(c_hbm, c_v, sems.at[0])
        d_wma = cp(wm_hbm.at[:, pl.ds(0, 2 * M)], wma_v, sems.at[1])
        d_x = cp(x_hbm, x_v, sems.at[2])
        d_wq = cp(wq_hbm, wq_v, sems.at[3])
        d_wuk = cp(wuk_hbm, wuk_v, sems.at[4])
        d_kv = lambda b: cp(ckv_hbm.at[b], ckv_v.at[b], ksems.at[b])
        d_wuv = cp(wuv_hbm, wuv_v, sems.at[5])
        d_wmb = cp(wm_hbm.at[:, pl.ds(2 * M, 4 * M)], wmb_v, sems.at[6])
        r = H * D // WO_CH
        d_wo = [cp(wo_hbm.at[pl.ds(i * r, r)], wo_v.at[pl.ds(i * r, r)], sems.at[7 + i]) for i in range(WO_CH)]
        d_w1 = cp(w1_hbm, w1_v, sems.at[7 + WO_CH])
        r2 = F // W2_CH
        d_w2 = [cp(w2_hbm.at[pl.ds(i * r2, r2)], w2_v.at[pl.ds(i * r2, r2)], sems.at[8 + WO_CH + i]) for i in range(W2_CH)]
        start = (lambda d: d.start()) if dma else (lambda d: None)
        wait = (lambda d: d.wait()) if dma else (lambda d: None)

        for d in [d_wma, d_c, d_x, d_wq, d_wuk]:
            start(d)

        wait(d_c)
        cc = c_v[...].astype(_F32)
        sc = (cc * jax.nn.sigmoid(cc)).astype(_BF16)
        wait(d_wma)
        moda = jnp.dot(sc, wma_v[...], preferred_element_type=_F32)
        wait(d_x)
        x = x_v[...].astype(_F32)
        h = (_layernorm(x) * (1.0 + moda[:, M:2 * M]) + moda[:, :M]).astype(_BF16)

        wait(d_wq)
        start(d_kv(0))
        wq32 = wq_v.bitcast(jnp.uint32)
        qs = []
        for j in range(HP):
            for w in _head_pair(wq32, j, M, HP):
                q = jnp.dot(h, w, preferred_element_type=_F32)
                qs.append((q * D ** -0.5).astype(_BF16))
        wait(d_wuk)
        start(d_kv(1))
        wuk32 = wuk_v.bitcast(jnp.uint32)
        for j in range(HP):
            for s, w in enumerate(_head_pair(wuk32, j, Dc, HP)):
                hh = 2 * j + s
                qa = jax.lax.dot_general(qs[hh], w, _NT, preferred_element_type=_F32)
                for n in range(NC):
                    qa_v[n, pl.ds(hh, B, stride=H), :] = qa[:, n * 128:(n + 1) * 128]

        def body(b, carry):
            wait(d_kv(b))

            @pl.when(b + 2 < B)
            def _():
                start(d_kv(b + 2))

            @pl.when(b + 2 == B)
            def _():
                start(d_wuv)

            @pl.when(b + 1 == B)
            def _():
                start(d_wmb)
                for d in d_wo:
                    start(d)

            row = pl.ds(pl.multiple_of(b * H, H), H)
            qa = jnp.concatenate([qa_v[n, row, :] for n in range(NC)], axis=1).astype(_BF16)
            s = jax.lax.dot_general(qa, ckv_v[b], _NT, preferred_element_type=_F32)
            m = jnp.max(s, axis=-1, keepdims=True)
            p = jnp.exp(s - m)
            l = jnp.sum(p, axis=-1, keepdims=True)
            o = jnp.dot(p.astype(_BF16), ckv_v[b], preferred_element_type=_F32) / l
            for n in range(NC):
                oc_v[n, row, :] = o[:, n * 128:(n + 1) * 128]
            return carry

        jax.lax.fori_loop(0, B, body, 0)

        wait(d_wuv)
        start(d_w1)
        wuv32 = wuv_v.bitcast(jnp.uint32)
        ctx = []
        for j in range(HP):
            for s, w in enumerate(_head_pair(wuv32, j, Dc, HP)):
                hh = 2 * j + s
                oc = jnp.concatenate([oc_v[n, pl.ds(hh, B, stride=H), :] for n in range(NC)], axis=1)
                ctx.append(jnp.dot(oc.astype(_BF16), w, preferred_element_type=_F32).astype(_BF16))
        wait(d_wmb)
        for d in d_w2:
            start(d)
        modb = jnp.dot(sc, wmb_v[...], preferred_element_type=_F32)
        att = None
        hc = H // WO_CH
        for i in range(WO_CH):
            wait(d_wo[i])
            t = jnp.dot(jnp.concatenate(ctx[i * hc:(i + 1) * hc], axis=1), wo_v[pl.ds(i * r, r), :],
                        preferred_element_type=_F32)
            att = t if att is None else att + t
        x1 = x + modb[:, :M] * att
        h2 = (_layernorm(x1) * (1.0 + modb[:, 2 * M:3 * M]) + modb[:, M:2 * M]).astype(_BF16)

        wait(d_w1)
        a = jnp.maximum(jnp.dot(h2, w1_v[...], preferred_element_type=_F32), 0.0).astype(_BF16)
        y = None
        for i in range(W2_CH):
            wait(d_w2[i])
            t = jnp.dot(a[:, i * r2:(i + 1) * r2], w2_v[pl.ds(i * r2, r2), :], preferred_element_type=_F32)
            y = t if y is None else y + t
        o_ref[...] = (x1 + modb[:, 3 * M:] * y).astype(o_ref.dtype)

    scratch = [
        pltpu.VMEM((B, M), _BF16), pltpu.VMEM((B, M), _BF16),
        pltpu.VMEM((B, Sk, Dc), _BF16),
        pltpu.VMEM((M * H, D), _BF16), pltpu.VMEM((Dc * H, D), _BF16), pltpu.VMEM((Dc * H, D), _BF16),
        pltpu.VMEM((H * D, M), _BF16), pltpu.VMEM((M, F), _BF16), pltpu.VMEM((F, M), _BF16),
        pltpu.VMEM((M, 2 * M), _BF16), pltpu.VMEM((M, 4 * M), _BF16),
        pltpu.VMEM((NC, B * H, 128), _F32), pltpu.VMEM((NC, B * H, 128), _F32),
        pltpu.SemaphoreType.DMA((8 + WO_CH + W2_CH,)), pltpu.SemaphoreType.DMA((B,)),
    ]
    return kernel, scratch


def _run(A_x, A_c_kv, A_w_q, A_w_uk, A_w_uv, A_w_o, B_w1, B_w2, c, w_mod, **kw):
    B, Sq, M = A_x.shape
    _, Sk, Dc = A_c_kv.shape
    _, H, D = A_w_q.shape
    F = B_w1.shape[1]
    kernel, scratch = _build(B, H, Sk, D, M, Dc, F, **kw)
    out = pl.pallas_call(
        kernel,
        out_shape=jax.ShapeDtypeStruct((B, M), A_x.dtype),
        in_specs=[pl.BlockSpec(memory_space=pl.ANY)] * 10,
        scratch_shapes=scratch,
        compiler_params=pltpu.CompilerParams(vmem_limit_bytes=100 * 1024 * 1024),
    )(A_x.reshape(B, M), A_c_kv, A_w_q.reshape(M * H, D), A_w_uk.reshape(Dc * H, D),
      A_w_uv.reshape(Dc * H, D), A_w_o.reshape(H * D, M), B_w1, B_w2, c, w_mod)
    return out.reshape(B, Sq, M)


@jax.jit
def pallas_adaLN_cond__compressed_kv_cla__dense_activation_relu__decode_kernel(
    A_x: jax.Array,
    A_c_kv: jax.Array,
    A_w_q: jax.Array,
    A_w_uk: jax.Array,
    A_w_uv: jax.Array,
    A_w_o: jax.Array,
    B_x: jax.Array,
    B_w1: jax.Array,
    B_w2: jax.Array,
    c: jax.Array,
    w_mod: jax.Array,
):
    return _run(A_x, A_c_kv, A_w_q, A_w_uk, A_w_uv, A_w_o, B_w1, B_w2, c, w_mod)
```

```python
import jax
import jax.numpy as jnp
import jax.experimental.pallas as pl
import jax.experimental.pallas.tpu as pltpu

_F32 = jnp.float32
_BF16 = jnp.bfloat16
_NT = (((1,), (1,)), ((), ()))


def _layernorm(x):
    m = jnp.mean(x, axis=-1, keepdims=True)
    d = x - m
    v = jnp.mean(d * d, axis=-1, keepdims=True)
    return d / jnp.sqrt(v + 1e-5)


def _head_pair(w32_ref, j, n, pairs):
    w = w32_ref[pl.ds(j, n, stride=pairs), :]
    lo = pltpu.bitcast(w << 16, _F32).astype(_BF16)
    hi = pltpu.bitcast(w & jnp.uint32(0xFFFF0000), _F32).astype(_BF16)
    return lo, hi


def _build(B, H, Sk, D, M, Dc, F, dma=True, WO_CH=4, W2_CH=7):
    HP = H // 2
    NC = Dc // 128

    def kernel(x_hbm, ckv_hbm, wq_hbm, wuk_hbm, wuv_hbm, wo_hbm, w1_hbm, w2_hbm, c_hbm, wm_hbm,
               o_ref,
               x_v, c_v, ckv_v, wq_v, wuk_v, wuv_v, wo_v, w1_v, w2_v, wma_v, wmb_v,
               qa_v, oc_v, fin_v, last_sem):
        def main(sems, ksems):
            cp = pltpu.make_async_copy
            d_c = cp(c_hbm, c_v, sems.at[0])
            d_wma = cp(wm_hbm.at[:, pl.ds(0, 2 * M)], wma_v, sems.at[1])
            d_x = cp(x_hbm, x_v, sems.at[2])
            d_wq = cp(wq_hbm, wq_v, sems.at[3])
            d_wuk = cp(wuk_hbm, wuk_v, sems.at[4])
            d_kv = lambda b: cp(ckv_hbm.at[b], ckv_v.at[b], ksems.at[b])
            d_wuv = cp(wuv_hbm, wuv_v, sems.at[5])
            d_wmb = cp(wm_hbm.at[:, pl.ds(2 * M, 4 * M)], wmb_v, sems.at[6])
            r = H * D // WO_CH
            d_wo = [cp(wo_hbm.at[pl.ds(i * r, r)], wo_v.at[pl.ds(i * r, r)], sems.at[7 + i]) for i in range(WO_CH)]
            d_w1 = cp(w1_hbm, w1_v, sems.at[7 + WO_CH])
            r2 = F // W2_CH
            d_w2 = [cp(w2_hbm.at[pl.ds(i * r2, r2)], w2_v.at[pl.ds(i * r2, r2)], sems.at[8 + WO_CH + i] if i < W2_CH - 1 else last_sem) for i in range(W2_CH)]
            start = (lambda d: d.start()) if dma else (lambda d: None)
            wait = (lambda d: d.wait()) if dma else (lambda d: None)

            for d in [d_wma, d_c, d_x, d_wq, d_wuk]:
                start(d)

            wait(d_c)
            cc = c_v[...].astype(_F32)
            sc = (cc * jax.nn.sigmoid(cc)).astype(_BF16)
            wait(d_wma)
            moda = jnp.dot(sc, wma_v[...], preferred_element_type=_F32)
            wait(d_x)
            x = x_v[...].astype(_F32)
            h = (_layernorm(x) * (1.0 + moda[:, M:2 * M]) + moda[:, :M]).astype(_BF16)

            wait(d_wq)
            start(d_kv(0))
            wq32 = wq_v.bitcast(jnp.uint32)
            qs = []
            for j in range(HP):
                for w in _head_pair(wq32, j, M, HP):
                    q = jnp.dot(h, w, preferred_element_type=_F32)
                    qs.append((q * D ** -0.5).astype(_BF16))
            wait(d_wuk)
            start(d_kv(1))
            wuk32 = wuk_v.bitcast(jnp.uint32)
            for j in range(HP):
                for s, w in enumerate(_head_pair(wuk32, j, Dc, HP)):
                    hh = 2 * j + s
                    qa = jax.lax.dot_general(qs[hh], w, _NT, preferred_element_type=_F32)
                    for n in range(NC):
                        qa_v[n, pl.ds(hh, B, stride=H), :] = qa[:, n * 128:(n + 1) * 128]

            def body(b, carry):
                wait(d_kv(b))

                @pl.when(b + 2 < B)
                def _():
                    start(d_kv(b + 2))

                @pl.when(b + 2 == B)
                def _():
                    start(d_wuv)

                @pl.when(b + 1 == B)
                def _():
                    start(d_wmb)
                    for d in d_wo:
                        start(d)

                row = pl.ds(pl.multiple_of(b * H, H), H)
                qa = jnp.concatenate([qa_v[n, row, :] for n in range(NC)], axis=1).astype(_BF16)
                s = jax.lax.dot_general(qa, ckv_v[b], _NT, preferred_element_type=_F32)
                m = jnp.max(s, axis=-1, keepdims=True)
                p = jnp.exp(s - m)
                l = jnp.sum(p, axis=-1, keepdims=True)
                o = jnp.dot(p.astype(_BF16), ckv_v[b], preferred_element_type=_F32) / l
                for n in range(NC):
                    oc_v[n, row, :] = o[:, n * 128:(n + 1) * 128]
                return carry

            jax.lax.fori_loop(0, B, body, 0)

            wait(d_wuv)
            start(d_w1)
            wuv32 = wuv_v.bitcast(jnp.uint32)
            ctx = []
            for j in range(HP):
                for s, w in enumerate(_head_pair(wuv32, j, Dc, HP)):
                    hh = 2 * j + s
                    oc = jnp.concatenate([oc_v[n, pl.ds(hh, B, stride=H), :] for n in range(NC)], axis=1)
                    ctx.append(jnp.dot(oc.astype(_BF16), w, preferred_element_type=_F32).astype(_BF16))
            wait(d_wmb)
            for d in d_w2:
                start(d)
            modb = jnp.dot(sc, wmb_v[...], preferred_element_type=_F32)
            att = None
            hc = H // WO_CH
            for i in range(WO_CH):
                wait(d_wo[i])
                t = jnp.dot(jnp.concatenate(ctx[i * hc:(i + 1) * hc], axis=1), wo_v[pl.ds(i * r, r), :],
                            preferred_element_type=_F32)
                att = t if att is None else att + t
            x1 = x + modb[:, :M] * att
            h2 = (_layernorm(x1) * (1.0 + modb[:, 2 * M:3 * M]) + modb[:, M:2 * M]).astype(_BF16)

            wait(d_w1)
            a = jnp.maximum(jnp.dot(h2, w1_v[...], preferred_element_type=_F32), 0.0).astype(_BF16)
            y = None
            for i in range(W2_CH - 1):
                wait(d_w2[i])
                t = jnp.dot(a[:, i * r2:(i + 1) * r2], w2_v[pl.ds(i * r2, r2), :], preferred_element_type=_F32)
                y = t if y is None else y + t
            gb = modb[:, 3 * M:]
            fin_v[:, :M] = x1 + gb * y
            fin_v[:, M:2 * M] = gb
            fin_v[:, 2 * M:] = a[:, F - r2:].astype(_F32)

        pl.run_scoped(
            main, pltpu.SemaphoreType.DMA((7 + WO_CH + W2_CH,)), pltpu.SemaphoreType.DMA((B,)))
        r2 = F // W2_CH
        last = pl.ds(F - r2, r2)
        base, gb, a_last = fin_v[:, :M], fin_v[:, M:2 * M], fin_v[:, 2 * M:].astype(_BF16)
        if dma:
            pltpu.make_async_copy(w2_hbm.at[last], w2_v.at[last], last_sem).wait()
        t = jnp.dot(a_last, w2_v[last, :], preferred_element_type=_F32)
        o_ref[...] = (base + gb * t).astype(o_ref.dtype)

    scratch = [
        pltpu.VMEM((B, M), _BF16), pltpu.VMEM((B, M), _BF16),
        pltpu.VMEM((B, Sk, Dc), _BF16),
        pltpu.VMEM((M * H, D), _BF16), pltpu.VMEM((Dc * H, D), _BF16), pltpu.VMEM((Dc * H, D), _BF16),
        pltpu.VMEM((H * D, M), _BF16), pltpu.VMEM((M, F), _BF16), pltpu.VMEM((F, M), _BF16),
        pltpu.VMEM((M, 2 * M), _BF16), pltpu.VMEM((M, 4 * M), _BF16),
        pltpu.VMEM((NC, B * H, 128), _F32), pltpu.VMEM((NC, B * H, 128), _F32),
        pltpu.VMEM((B, 2 * M + F // W2_CH), _F32),
        pltpu.SemaphoreType.DMA(()),
    ]
    return kernel, scratch


def _run(A_x, A_c_kv, A_w_q, A_w_uk, A_w_uv, A_w_o, B_w1, B_w2, c, w_mod, cpk={}, **kw):
    B, Sq, M = A_x.shape
    _, Sk, Dc = A_c_kv.shape
    _, H, D = A_w_q.shape
    F = B_w1.shape[1]
    kernel, scratch = _build(B, H, Sk, D, M, Dc, F, **kw)
    out = pl.pallas_call(
        kernel,
        out_shape=jax.ShapeDtypeStruct((B, M), A_x.dtype),
        in_specs=[pl.BlockSpec(memory_space=pl.ANY)] * 10,
        scratch_shapes=scratch,
        compiler_params=pltpu.CompilerParams(vmem_limit_bytes=100 * 1024 * 1024, **cpk),
    )(A_x.reshape(B, M), A_c_kv, A_w_q.reshape(M * H, D), A_w_uk.reshape(Dc * H, D),
      A_w_uv.reshape(Dc * H, D), A_w_o.reshape(H * D, M), B_w1, B_w2, c, w_mod)
    return out.reshape(B, Sq, M)


@jax.jit
def pallas_adaLN_cond__compressed_kv_cla__dense_activation_relu__decode_kernel(
    A_x: jax.Array,
    A_c_kv: jax.Array,
    A_w_q: jax.Array,
    A_w_uk: jax.Array,
    A_w_uv: jax.Array,
    A_w_o: jax.Array,
    B_x: jax.Array,
    B_w1: jax.Array,
    B_w2: jax.Array,
    c: jax.Array,
    w_mod: jax.Array,
):
    return _run(A_x, A_c_kv, A_w_q, A_w_uk, A_w_uv, A_w_o, B_w1, B_w2, c, w_mod)
```

```python
import jax
import jax.numpy as jnp
import jax.experimental.pallas as pl
import jax.experimental.pallas.tpu as pltpu

_F32 = jnp.float32
_BF16 = jnp.bfloat16
_NT = (((1,), (1,)), ((), ()))
_PIECE = 16 * 1024


def _layernorm(x):
    m = jnp.mean(x, axis=-1, keepdims=True)
    d = x - m
    v = jnp.mean(d * d, axis=-1, keepdims=True)
    return d / jnp.sqrt(v + 1e-5)


def _head_pair(w32_ref, j, pairs):
    s, rows, d = w32_ref.shape
    w = w32_ref[:, pl.ds(j, rows // pairs, stride=pairs), :].reshape(s * rows // pairs, d)
    lo = pltpu.bitcast(w << 16, _F32).astype(_BF16)
    hi = pltpu.bitcast(w & jnp.uint32(0xFFFF0000), _F32).astype(_BF16)
    return lo, hi


def _stream(copies, part=0, parts=1):
    streams, rows, cols = copies[0][0].shape
    steps = rows * cols * 2 // _PIECE

    def step(i, carry):
        k = 0
        for src, dst, sem in copies:
            r = src.shape[1] // steps
            for s in range(0, streams, 2):
                idx = (pl.ds(s, 2), pl.ds(pl.multiple_of(i * r, r), r))
                pltpu.make_async_copy(src.at[idx], dst.at[idx], sem).start(priority=k % 2)
                k += 1
        return carry

    jax.lax.fori_loop(part * steps // parts, (part + 1) * steps // parts, step, 0)


def _stream_rows(src, dst, sem, r, streams):
    per = src.shape[0] // streams

    def step(i, carry):
        for s in range(streams):
            idx = pl.ds(pl.multiple_of(s * per + i * r, r), r)
            pltpu.make_async_copy(src.at[idx], dst.at[idx], sem).start(priority=s % 2)
        return carry

    jax.lax.fori_loop(0, per // r, step, 0)


def _wait(dst, sem):
    pltpu.make_async_copy(dst, dst, sem).wait()


def _build(B, H, Sk, D, M, Dc, F, S):
    HP = H // 2
    NC = Dc // 128
    R2 = 128
    N2 = F // R2

    def kernel(x_hbm, ckv_hbm, wq_hbm, wuk_hbm, wuv_hbm, wo_hbm, w1_hbm, w2_hbm, c_hbm, wm_hbm,
               o_ref,
               x_v, c_v, ckv_v, wq_v, wuk_v, wuv_v, wo_v, w1_v, w2_v, wma_v, wmb_v,
               qa_v, oc_v, fin_v, last_sem):

        def main(sems, ksems, fsems):
            s_c, s_x, s_wma, s_wq, s_wuk, s_wuv, s_wo, s_wmb, s_w1 = (sems.at[i] for i in range(9))
            kv = lambda b: (ckv_hbm.at[b], ckv_v.at[b], ksems.at[b])

            pltpu.make_async_copy(c_hbm, c_v, s_c).start()
            pltpu.make_async_copy(x_hbm, x_v, s_x).start(priority=1)
            _stream_rows(wm_hbm.at[:, pl.ds(0, 2 * M)], wma_v, s_wma, 16, 8)
            _stream([(wq_hbm, wq_v, s_wq)])

            _wait(c_v, s_c)
            cc = c_v[...].astype(_F32)
            sc = (cc * jax.nn.sigmoid(cc)).astype(_BF16)
            _wait(wma_v, s_wma)
            moda = jnp.dot(sc, wma_v[...], preferred_element_type=_F32)
            _wait(x_v, s_x)
            x = x_v[...].astype(_F32)
            h = (_layernorm(x) * (1.0 + moda[:, M:]) + moda[:, :M]).astype(_BF16)

            _stream([(wuk_hbm, wuk_v, s_wuk)], 0, 2)
            _wait(wq_v, s_wq)
            wq32 = wq_v.bitcast(jnp.uint32)
            qs = []
            for j in range(HP):
                if j == HP // 2:
                    _stream([(wuk_hbm, wuk_v, s_wuk)], 1, 2)
                for w in _head_pair(wq32, j, HP):
                    q = jnp.dot(h, w, preferred_element_type=_F32)
                    qs.append((q * D ** -0.5).astype(_BF16))
            _stream([kv(0)], 0, 2)
            _wait(wuk_v, s_wuk)
            wuk32 = wuk_v.bitcast(jnp.uint32)
            for j in range(HP):
                if j == HP // 2:
                    _stream([kv(0)], 1, 2)
                for s, w in enumerate(_head_pair(wuk32, j, HP)):
                    hh = 2 * j + s
                    qa = jax.lax.dot_general(qs[hh], w, _NT, preferred_element_type=_F32)
                    for n in range(NC):
                        qa_v[n, pl.ds(hh, B, stride=H), :] = qa[:, n * 128:(n + 1) * 128]

            def body(b, carry):
                @pl.when(b + 1 < B)
                def _():
                    _stream([kv(b + 1)])

                @pl.when(b + 1 == B)
                def _():
                    _stream([(wuv_hbm, wuv_v, s_wuv)])

                _wait(ckv_v.at[b], ksems.at[b])
                row = pl.ds(pl.multiple_of(b * H, H), H)
                qa = jnp.concatenate([qa_v[n, row, :] for n in range(NC)], axis=1).astype(_BF16)
                s = jax.lax.dot_general(qa, ckv_v[b].reshape(Sk, Dc), _NT, preferred_element_type=_F32)
                m = jnp.max(s, axis=-1, keepdims=True)
                p = jnp.exp(s - m)
                l = jnp.sum(p, axis=-1, keepdims=True)
                o = jnp.dot(p.astype(_BF16), ckv_v[b].reshape(Sk, Dc), preferred_element_type=_F32) / l
                for n in range(NC):
                    oc_v[n, row, :] = o[:, n * 128:(n + 1) * 128]
                return carry

            jax.lax.fori_loop(0, B, body, 0)

            _stream([(wo_hbm, wo_v, s_wo)], 0, 2)
            _wait(wuv_v, s_wuv)
            wuv32 = wuv_v.bitcast(jnp.uint32)
            ctx = []
            for j in range(HP):
                if j == HP // 2:
                    _stream([(wo_hbm, wo_v, s_wo)], 1, 2)
                for s, w in enumerate(_head_pair(wuv32, j, HP)):
                    hh = 2 * j + s
                    oc = jnp.concatenate([oc_v[n, pl.ds(hh, B, stride=H), :] for n in range(NC)], axis=1)
                    ctx.append(jnp.dot(oc.astype(_BF16), w, preferred_element_type=_F32).astype(_BF16))
            _stream_rows(wm_hbm.at[:, pl.ds(2 * M, 4 * M)], wmb_v, s_wmb, 8, 8)
            _wait(wo_v, s_wo)
            att = jnp.dot(jnp.concatenate(ctx, axis=1), wo_v[...].reshape(H * D, M),
                          preferred_element_type=_F32)
            _stream_rows(w1_hbm, w1_v, s_w1, 8, 8)
            _wait(wmb_v, s_wmb)
            modb = jnp.dot(sc, wmb_v[...], preferred_element_type=_F32)
            x1 = x + modb[:, :M] * att
            h2 = (_layernorm(x1) * (1.0 + modb[:, 2 * M:3 * M]) + modb[:, M:2 * M]).astype(_BF16)

            for i in range(N2):
                for k in range(R2 // 32):
                    idx = pl.ds(i * R2 + k * 32, 32)
                    sem = fsems.at[i] if i < N2 - 1 else last_sem
                    pltpu.make_async_copy(w2_hbm.at[idx], w2_v.at[idx], sem).start(priority=k % 2)
            _wait(w1_v, s_w1)
            a = jnp.maximum(jnp.dot(h2, w1_v[...], preferred_element_type=_F32), 0.0)
            y = None
            for i in range(N2 - 1):
                idx = pl.ds(i * R2, R2)
                _wait(w2_v.at[idx], fsems.at[i])
                t = jnp.dot(a[:, i * R2:(i + 1) * R2].astype(_BF16), w2_v[idx, :], preferred_element_type=_F32)
                y = t if y is None else y + t
            gb = modb[:, 3 * M:]
            fin_v[:, :M] = x1 + gb * y
            fin_v[:, M:2 * M] = gb
            fin_v[:, 2 * M:] = a[:, F - R2:]

        pl.run_scoped(main, pltpu.SemaphoreType.DMA((9,)), pltpu.SemaphoreType.DMA((B,)),
                      pltpu.SemaphoreType.DMA((N2 - 1,)))
        last = pl.ds(F - R2, R2)
        base, gb, a_last = fin_v[:, :M], fin_v[:, M:2 * M], fin_v[:, 2 * M:].astype(_BF16)
        _wait(w2_v.at[last], last_sem)
        t = jnp.dot(a_last, w2_v[last, :], preferred_element_type=_F32)
        o_ref[...] = (base + gb * t).astype(o_ref.dtype)

    scratch = [
        pltpu.VMEM((B, M), _BF16), pltpu.VMEM((B, M), _BF16),
        pltpu.VMEM((B, S, Sk // S, Dc), _BF16),
        pltpu.VMEM((S, M * H // S, D), _BF16), pltpu.VMEM((S, Dc * H // S, D), _BF16),
        pltpu.VMEM((S, Dc * H // S, D), _BF16), pltpu.VMEM((S, H * D // S, M), _BF16),
        pltpu.VMEM((M, F), _BF16), pltpu.VMEM((F, M), _BF16),
        pltpu.VMEM((M, 2 * M), _BF16), pltpu.VMEM((M, 4 * M), _BF16),
        pltpu.VMEM((NC, B * H, 128), _F32), pltpu.VMEM((NC, B * H, 128), _F32),
        pltpu.VMEM((B, 2 * M + R2), _F32),
        pltpu.SemaphoreType.DMA(()),
    ]
    return kernel, scratch


def _run(A_x, A_c_kv, A_w_q, A_w_uk, A_w_uv, A_w_o, B_w1, B_w2, c, w_mod, S=8):
    B, Sq, M = A_x.shape
    _, Sk, Dc = A_c_kv.shape
    _, H, D = A_w_q.shape
    F = B_w1.shape[1]
    assert Sq == 1
    kernel, scratch = _build(B, H, Sk, D, M, Dc, F, S)
    out = pl.pallas_call(
        kernel,
        out_shape=jax.ShapeDtypeStruct((B, M), A_x.dtype),
        in_specs=[pl.BlockSpec(memory_space=pl.ANY)] * 10,
        scratch_shapes=scratch,
        compiler_params=pltpu.CompilerParams(vmem_limit_bytes=100 * 1024 * 1024),
    )(A_x.reshape(B, M), A_c_kv.reshape(B, S, Sk // S, Dc), A_w_q.reshape(S, -1, D),
      A_w_uk.reshape(S, -1, D), A_w_uv.reshape(S, -1, D), A_w_o.reshape(S, -1, M), B_w1, B_w2, c, w_mod)
    return out.reshape(B, Sq, M)


@jax.jit
def pallas_adaLN_cond__compressed_kv_cla__dense_activation_relu__decode_kernel(
    A_x: jax.Array,
    A_c_kv: jax.Array,
    A_w_q: jax.Array,
    A_w_uk: jax.Array,
    A_w_uv: jax.Array,
    A_w_o: jax.Array,
    B_x: jax.Array,
    B_w1: jax.Array,
    B_w2: jax.Array,
    c: jax.Array,
    w_mod: jax.Array,
):
    del B_x
    return _run(A_x, A_c_kv, A_w_q, A_w_uk, A_w_uv, A_w_o, B_w1, B_w2, c, w_mod)
```

```python
import jax
import jax.numpy as jnp
import jax.experimental.pallas as pl
import jax.experimental.pallas.tpu as pltpu

_F32 = jnp.float32
_BF16 = jnp.bfloat16
_NT = (((1,), (1,)), ((), ()))
_PIECE = 16 * 1024


def _layernorm(x):
    m = jnp.mean(x, axis=-1, keepdims=True)
    d = x - m
    v = jnp.mean(d * d, axis=-1, keepdims=True)
    return d / jnp.sqrt(v + 1e-5)


def _head_pair(w32_ref, j, pairs):
    s, rows, d = w32_ref.shape
    w = w32_ref[:, pl.ds(j, rows // pairs, stride=pairs), :].reshape(s * rows // pairs, d)
    lo = pltpu.bitcast(w << 16, _F32).astype(_BF16)
    hi = pltpu.bitcast(w & jnp.uint32(0xFFFF0000), _F32).astype(_BF16)
    return lo, hi


def _stream(copies, part=0, parts=1):
    streams, rows, cols = copies[0][0].shape
    steps = rows * cols * 2 // _PIECE

    def step(i, carry):
        k = 0
        for src, dst, sem in copies:
            r = src.shape[1] // steps
            for s in range(0, streams, 2):
                idx = (pl.ds(s, 2), pl.ds(pl.multiple_of(i * r, r), r))
                pltpu.make_async_copy(src.at[idx], dst.at[idx], sem).start(priority=k % 2)
                k += 1
        return carry

    jax.lax.fori_loop(part * steps // parts, (part + 1) * steps // parts, step, 0)


def _stream_rows(src, dst, sem, r, streams):
    per = src.shape[0] // streams

    def step(i, carry):
        for s in range(streams):
            idx = pl.ds(pl.multiple_of(s * per + i * r, r), r)
            pltpu.make_async_copy(src.at[idx], dst.at[idx], sem).start(priority=s % 2)
        return carry

    jax.lax.fori_loop(0, per // r, step, 0)


def _wait(dst, sem):
    pltpu.make_async_copy(dst, dst, sem).wait()


def _build(B, H, Sk, D, M, Dc, F, S):
    HP = H // 2
    NC = Dc // 128
    R2 = 128
    N2 = F // R2

    def kernel(x_hbm, ckv_hbm, wq_hbm, wuk_hbm, wuv_hbm, wo_hbm, w1_hbm, w2_hbm, c_hbm, wm_hbm,
               o_ref,
               x_v, c_v, ckv_v, wq_v, wuk_v, wuv_v, wo_v, w1_v, w2_v, wma_v, wmb_v,
               qa_v, oc_v, fin_v, last_sem):

        def main(sems, ksems, fsems):
            s_c, s_x, s_wma, s_wq, s_wuk, s_wuv, s_wo, s_wmb, s_w1 = (sems.at[i] for i in range(9))
            kv = lambda b: (ckv_hbm.at[b], ckv_v.at[b], ksems.at[b])

            pltpu.make_async_copy(c_hbm, c_v, s_c).start()
            pltpu.make_async_copy(x_hbm, x_v, s_x).start(priority=1)
            _stream_rows(wm_hbm.at[:, pl.ds(0, 2 * M)], wma_v, s_wma, 16, 8)
            _stream([(wq_hbm, wq_v, s_wq)])

            _wait(c_v, s_c)
            cc = c_v[...].astype(_F32)
            sc = (cc * jax.nn.sigmoid(cc)).astype(_BF16)
            _wait(wma_v, s_wma)
            moda = jnp.dot(sc, wma_v[...], preferred_element_type=_F32)
            _wait(x_v, s_x)
            x = x_v[...].astype(_F32)
            h = (_layernorm(x) * (1.0 + moda[:, M:]) + moda[:, :M]).astype(_BF16)

            _stream([(wuk_hbm, wuk_v, s_wuk)])
            _wait(wq_v, s_wq)
            wq32 = wq_v.bitcast(jnp.uint32)
            qs = []
            for j in range(HP):
                if j == HP // 2:
                    _stream([kv(0)], 0, 2)
                for w in _head_pair(wq32, j, HP):
                    q = jnp.dot(h, w, preferred_element_type=_F32)
                    qs.append((q * D ** -0.5).astype(_BF16))
            _stream([kv(0)], 1, 2)
            _wait(wuk_v, s_wuk)
            wuk32 = wuk_v.bitcast(jnp.uint32)
            for j in range(HP):
                if j == HP // 2:
                    _stream([kv(1)], 0, 2)
                for s, w in enumerate(_head_pair(wuk32, j, HP)):
                    hh = 2 * j + s
                    qa = jax.lax.dot_general(qs[hh], w, _NT, preferred_element_type=_F32)
                    for n in range(NC):
                        qa_v[n, pl.ds(hh, B, stride=H), :] = qa[:, n * 128:(n + 1) * 128]

            def body(b, carry):
                _wait(ckv_v.at[b], ksems.at[b])
                row = pl.ds(pl.multiple_of(b * H, H), H)
                qa = jnp.concatenate([qa_v[n, row, :] for n in range(NC)], axis=1).astype(_BF16)
                s = jax.lax.dot_general(qa, ckv_v[b].reshape(Sk, Dc), _NT, preferred_element_type=_F32)
                m = jnp.max(s, axis=-1, keepdims=True)
                p = jnp.exp(s - m)
                l = jnp.sum(p, axis=-1, keepdims=True)
                o = jnp.dot(p.astype(_BF16), ckv_v[b].reshape(Sk, Dc), preferred_element_type=_F32) / l
                for n in range(NC):
                    oc_v[n, row, :] = o[:, n * 128:(n + 1) * 128]

                @pl.when(b + 2 < B)
                def _():
                    _stream([kv(b + 2)])

                @pl.when(b + 2 == B)
                def _():
                    _stream([(wuv_hbm, wuv_v, s_wuv)])

                return carry

            _stream([kv(1)], 1, 2)
            jax.lax.fori_loop(0, B, body, 0)

            _stream([(wo_hbm, wo_v, s_wo)])
            _wait(wuv_v, s_wuv)
            wuv32 = wuv_v.bitcast(jnp.uint32)
            ctx = []
            for j in range(HP):
                if j == HP // 2:
                    _stream_rows(wm_hbm.at[:, pl.ds(2 * M, 4 * M)], wmb_v, s_wmb, 8, 8)
                for s, w in enumerate(_head_pair(wuv32, j, HP)):
                    hh = 2 * j + s
                    oc = jnp.concatenate([oc_v[n, pl.ds(hh, B, stride=H), :] for n in range(NC)], axis=1)
                    ctx.append(jnp.dot(oc.astype(_BF16), w, preferred_element_type=_F32).astype(_BF16))
            _stream_rows(w1_hbm, w1_v, s_w1, 8, 8)
            _wait(wo_v, s_wo)
            att = jnp.dot(jnp.concatenate(ctx, axis=1), wo_v[...].reshape(H * D, M),
                          preferred_element_type=_F32)
            for i in range(N2):
                for k in range(R2 // 32):
                    idx = pl.ds(i * R2 + k * 32, 32)
                    sem = fsems.at[i] if i < N2 - 1 else last_sem
                    pltpu.make_async_copy(w2_hbm.at[idx], w2_v.at[idx], sem).start(priority=k % 2)
            _wait(wmb_v, s_wmb)
            modb = jnp.dot(sc, wmb_v[...], preferred_element_type=_F32)
            x1 = x + modb[:, :M] * att
            h2 = (_layernorm(x1) * (1.0 + modb[:, 2 * M:3 * M]) + modb[:, M:2 * M]).astype(_BF16)

            _wait(w1_v, s_w1)
            a = jnp.maximum(jnp.dot(h2, w1_v[...], preferred_element_type=_F32), 0.0)
            y = None
            for i in range(N2 - 1):
                idx = pl.ds(i * R2, R2)
                _wait(w2_v.at[idx], fsems.at[i])
                t = jnp.dot(a[:, i * R2:(i + 1) * R2].astype(_BF16), w2_v[idx, :], preferred_element_type=_F32)
                y = t if y is None else y + t
            gb = modb[:, 3 * M:]
            fin_v[:, :M] = x1 + gb * y
            fin_v[:, M:2 * M] = gb
            fin_v[:, 2 * M:] = a[:, F - R2:]

        pl.run_scoped(main, pltpu.SemaphoreType.DMA((9,)), pltpu.SemaphoreType.DMA((B,)),
                      pltpu.SemaphoreType.DMA((N2 - 1,)))
        last = pl.ds(F - R2, R2)
        base, gb, a_last = fin_v[:, :M], fin_v[:, M:2 * M], fin_v[:, 2 * M:].astype(_BF16)
        _wait(w2_v.at[last], last_sem)
        t = jnp.dot(a_last, w2_v[last, :], preferred_element_type=_F32)
        o_ref[...] = (base + gb * t).astype(o_ref.dtype)

    scratch = [
        pltpu.VMEM((B, M), _BF16), pltpu.VMEM((B, M), _BF16),
        pltpu.VMEM((B, S, Sk // S, Dc), _BF16),
        pltpu.VMEM((S, M * H // S, D), _BF16), pltpu.VMEM((S, Dc * H // S, D), _BF16),
        pltpu.VMEM((S, Dc * H // S, D), _BF16), pltpu.VMEM((S, H * D // S, M), _BF16),
        pltpu.VMEM((M, F), _BF16), pltpu.VMEM((F, M), _BF16),
        pltpu.VMEM((M, 2 * M), _BF16), pltpu.VMEM((M, 4 * M), _BF16),
        pltpu.VMEM((NC, B * H, 128), _F32), pltpu.VMEM((NC, B * H, 128), _F32),
        pltpu.VMEM((B, 2 * M + R2), _F32),
        pltpu.SemaphoreType.DMA(()),
    ]
    return kernel, scratch


def _run(A_x, A_c_kv, A_w_q, A_w_uk, A_w_uv, A_w_o, B_w1, B_w2, c, w_mod, S=8):
    B, Sq, M = A_x.shape
    _, Sk, Dc = A_c_kv.shape
    _, H, D = A_w_q.shape
    F = B_w1.shape[1]
    assert Sq == 1
    kernel, scratch = _build(B, H, Sk, D, M, Dc, F, S)
    out = pl.pallas_call(
        kernel,
        out_shape=jax.ShapeDtypeStruct((B, M), A_x.dtype),
        in_specs=[pl.BlockSpec(memory_space=pl.ANY)] * 10,
        scratch_shapes=scratch,
        compiler_params=pltpu.CompilerParams(vmem_limit_bytes=100 * 1024 * 1024),
    )(A_x.reshape(B, M), A_c_kv.reshape(B, S, Sk // S, Dc), A_w_q.reshape(S, -1, D),
      A_w_uk.reshape(S, -1, D), A_w_uv.reshape(S, -1, D), A_w_o.reshape(S, -1, M), B_w1, B_w2, c, w_mod)
    return out.reshape(B, Sq, M)


@jax.jit
def pallas_adaLN_cond__compressed_kv_cla__dense_activation_relu__decode_kernel(
    A_x: jax.Array,
    A_c_kv: jax.Array,
    A_w_q: jax.Array,
    A_w_uk: jax.Array,
    A_w_uv: jax.Array,
    A_w_o: jax.Array,
    B_x: jax.Array,
    B_w1: jax.Array,
    B_w2: jax.Array,
    c: jax.Array,
    w_mod: jax.Array,
):
    del B_x
    return _run(A_x, A_c_kv, A_w_q, A_w_uk, A_w_uv, A_w_o, B_w1, B_w2, c, w_mod)
```

```python
import jax
import jax.numpy as jnp
import jax.experimental.pallas as pl
import jax.experimental.pallas.tpu as pltpu

_F32 = jnp.float32
_BF16 = jnp.bfloat16
_NT = (((1,), (1,)), ((), ()))
_PRIO = (1, 1, 1, 0)
_PIECE = 16 * 1024


def _layernorm(x):
    m = jnp.mean(x, axis=-1, keepdims=True)
    d = x - m
    v = jnp.mean(d * d, axis=-1, keepdims=True)
    return d / jnp.sqrt(v + 1e-5)


def _head_pair(w32_ref, j, pairs):
    s, rows, d = w32_ref.shape
    w = w32_ref[:, pl.ds(j, rows // pairs, stride=pairs), :].reshape(s * rows // pairs, d)
    lo = pltpu.bitcast(w << 16, _F32).astype(_BF16)
    hi = pltpu.bitcast(w & jnp.uint32(0xFFFF0000), _F32).astype(_BF16)
    return lo, hi


def _stream(copies, part=0, parts=1):
    streams, rows, cols = copies[0][0].shape
    steps = rows * cols * 2 // _PIECE

    def step(i, carry):
        k = 0
        for src, dst, sem in copies:
            r = src.shape[1] // steps
            for s in range(0, streams, 2):
                idx = (pl.ds(s, 2), pl.ds(pl.multiple_of(i * r, r), r))
                pltpu.make_async_copy(src.at[idx], dst.at[idx], sem).start(priority=_PRIO[k % len(_PRIO)])
                k += 1
        return carry

    jax.lax.fori_loop(part * (steps // parts), (part + 1) * (steps // parts), step, 0)


def _stream_rows(src, dst, sem, r, streams, prio=(0, 1), part=0, parts=1):
    per = src.shape[0] // streams

    def step(i, carry):
        for s in range(streams):
            idx = pl.ds(pl.multiple_of(s * per + i * r, r), r)
            pltpu.make_async_copy(src.at[idx], dst.at[idx], sem).start(priority=prio[s % len(prio)])
        return carry

    n = per // r // parts
    jax.lax.fori_loop(part * n, (part + 1) * n, step, 0)


def _wait(dst, sem):
    pltpu.make_async_copy(dst, dst, sem).wait()


def _build(B, H, Sk, D, M, Dc, F, S, pa=_PRIO, pb=_PRIO, p1=_PRIO, p2=_PRIO, W2=(768, 512, 256, 256), E1=0):
    HP = H // 2
    NC = Dc // 128
    N2 = len(W2)
    R2 = W2[-1]
    O2 = [sum(W2[:i]) for i in range(N2)]

    def kernel(x_hbm, ckv_hbm, wq_hbm, wuk_hbm, wuv_hbm, wo_hbm, w1_hbm, w2_hbm, c_hbm, wm_hbm,
               o_ref,
               x_v, c_v, ckv_v, wq_v, wuk_v, wuv_v, wo_v, w1_v, w2_v, wma_v, wmb_v,
               qa_v, oc_v, fin_v, last_sem):

        def main(sems, ksems, fsems):
            s_c, s_x, s_wma, s_wq, s_wuk, s_wuv, s_wo, s_wmb, s_w1 = (sems.at[i] for i in range(9))
            kv = lambda g: [(ckv_hbm.at[2 * g + i], ckv_v.at[2 * g + i], ksems.at[2 * g + i]) for i in range(2)]
            wqk = [(wq_hbm, wq_v, s_wq), (wuk_hbm, wuk_v, s_wuk)]
            wvo = [(wuv_hbm, wuv_v, s_wuv), (wo_hbm, wo_v, s_wo)]


            def start_w2(lo, hi):
                for r in range(lo, hi, 32):
                    i = max(k for k in range(N2) if O2[k] <= r)
                    idx = pl.ds(r, 32)
                    sem = fsems.at[i] if i < N2 - 1 else last_sem
                    pltpu.make_async_copy(w2_hbm.at[idx], w2_v.at[idx], sem).start(priority=p2[r // 32 % len(p2)])

            pltpu.make_async_copy(c_hbm, c_v, s_c).start()
            pltpu.make_async_copy(x_hbm, x_v, s_x).start(priority=1)
            _stream_rows(wm_hbm.at[:, pl.ds(0, 2 * M)], wma_v, s_wma, 16, 8, pa)
            _stream(wqk)

            _wait(c_v, s_c)
            cc = c_v[...].astype(_F32)
            sc = (cc * jax.nn.sigmoid(cc)).astype(_BF16)
            _wait(wma_v, s_wma)
            moda = jnp.dot(sc, wma_v[...], preferred_element_type=_F32)
            _wait(x_v, s_x)
            x = x_v[...].astype(_F32)
            h = (_layernorm(x) * (1.0 + moda[:, M:]) + moda[:, :M]).astype(_BF16)

            _stream(kv(0), 0, 2)
            _wait(wq_v, s_wq)
            wq32 = wq_v.bitcast(jnp.uint32)
            qs = []
            for j in range(HP):
                if j == HP // 2:
                    _stream(kv(0), 2, 4)
                for w in _head_pair(wq32, j, HP):
                    q = jnp.dot(h, w, preferred_element_type=_F32)
                    qs.append((q * D ** -0.5).astype(_BF16))
            _stream(kv(0), 3, 4)
            _wait(wuk_v, s_wuk)
            wuk32 = wuk_v.bitcast(jnp.uint32)
            for j in range(HP):
                if j == HP // 2:
                    _stream(kv(1), 0, 4)
                for s, w in enumerate(_head_pair(wuk32, j, HP)):
                    hh = 2 * j + s
                    qa = jax.lax.dot_general(qs[hh], w, _NT, preferred_element_type=_F32)
                    for n in range(NC):
                        qa_v[n, pl.ds(hh, B, stride=H), :] = qa[:, n * 128:(n + 1) * 128]

            def body(b, carry):
                _wait(ckv_v.at[b], ksems.at[b])
                row = pl.ds(pl.multiple_of(b * H, H), H)
                qa = jnp.concatenate([qa_v[n, row, :] for n in range(NC)], axis=1).astype(_BF16)
                s = jax.lax.dot_general(qa, ckv_v[b].reshape(Sk, Dc), _NT, preferred_element_type=_F32)
                m = jnp.max(s, axis=-1, keepdims=True)
                p = jnp.exp(s - m)
                l = jnp.sum(p, axis=-1, keepdims=True)
                o = jnp.dot(p.astype(_BF16), ckv_v[b].reshape(Sk, Dc), preferred_element_type=_F32) / l
                for n in range(NC):
                    oc_v[n, row, :] = o[:, n * 128:(n + 1) * 128]

                t = b + 3

                @pl.when(t < B)
                def _():
                    _stream(kv(t // 2), t % 2, 2)

                @pl.when(jnp.logical_and(t >= B, t < B + 2))
                def _():
                    _stream(wvo, t % 2, 2)

                return carry

            _stream(kv(1), 1, 4)
            jax.lax.fori_loop(0, B, body, 0)

            _stream_rows(wm_hbm.at[:, pl.ds(2 * M, 4 * M)], wmb_v, s_wmb, 8, 8, pb)
            for k in range(E1):
                _stream_rows(w1_hbm, w1_v, s_w1, 8, 8, p1, k, 4)
            _wait(wuv_v, s_wuv)
            wuv32 = wuv_v.bitcast(jnp.uint32)
            ctx = []
            for j in range(HP):
                if j % 4 == 0 and E1 + j // 4 < 4:
                    _stream_rows(w1_hbm, w1_v, s_w1, 8, 8, p1, E1 + j // 4, 4)
                if j % 4 == 0 and E1 + j // 4 >= 4:
                    start_w2((E1 + j // 4 - 4) * 448, (E1 + j // 4 - 3) * 448)
                for s, w in enumerate(_head_pair(wuv32, j, HP)):
                    hh = 2 * j + s
                    oc = jnp.concatenate([oc_v[n, pl.ds(hh, B, stride=H), :] for n in range(NC)], axis=1)
                    ctx.append(jnp.dot(oc.astype(_BF16), w, preferred_element_type=_F32).astype(_BF16))
            start_w2(E1 * 448, F)
            _wait(wo_v, s_wo)
            att = jnp.dot(jnp.concatenate(ctx, axis=1), wo_v[...].reshape(H * D, M),
                          preferred_element_type=_F32)
            _wait(wmb_v, s_wmb)
            modb = jnp.dot(sc, wmb_v[...], preferred_element_type=_F32)
            x1 = x + modb[:, :M] * att
            h2 = (_layernorm(x1) * (1.0 + modb[:, 2 * M:3 * M]) + modb[:, M:2 * M]).astype(_BF16)

            _wait(w1_v, s_w1)
            a = jnp.maximum(jnp.dot(h2, w1_v[...], preferred_element_type=_F32), 0.0)
            y = None
            for i in range(N2 - 1):
                idx = pl.ds(O2[i], W2[i])
                _wait(w2_v.at[idx], fsems.at[i])
                t = jnp.dot(a[:, O2[i]:O2[i] + W2[i]].astype(_BF16), w2_v[idx, :], preferred_element_type=_F32)
                y = t if y is None else y + t
            gb = modb[:, 3 * M:]
            fin_v[:, :M] = x1 + gb * y
            fin_v[:, M:2 * M] = gb
            fin_v[:, 2 * M:] = a[:, F - R2:]

        pl.run_scoped(main, pltpu.SemaphoreType.DMA((9,)), pltpu.SemaphoreType.DMA((B,)),
                      pltpu.SemaphoreType.DMA((N2 - 1,)))
        last = pl.ds(F - R2, R2)
        base, gb, a_last = fin_v[:, :M], fin_v[:, M:2 * M], fin_v[:, 2 * M:].astype(_BF16)
        _wait(w2_v.at[last], last_sem)
        t = jnp.dot(a_last, w2_v[last, :], preferred_element_type=_F32)
        o_ref[...] = (base + gb * t).astype(o_ref.dtype)

    scratch = [
        pltpu.VMEM((B, M), _BF16), pltpu.VMEM((B, M), _BF16),
        pltpu.VMEM((B, S, Sk // S, Dc), _BF16),
        pltpu.VMEM((S, M * H // S, D), _BF16), pltpu.VMEM((S, Dc * H // S, D), _BF16),
        pltpu.VMEM((S, Dc * H // S, D), _BF16), pltpu.VMEM((S, H * D // S, M), _BF16),
        pltpu.VMEM((M, F), _BF16), pltpu.VMEM((F, M), _BF16),
        pltpu.VMEM((M, 2 * M), _BF16), pltpu.VMEM((M, 4 * M), _BF16),
        pltpu.VMEM((NC, B * H, 128), _F32), pltpu.VMEM((NC, B * H, 128), _F32),
        pltpu.VMEM((B, 2 * M + R2), _F32),
        pltpu.SemaphoreType.DMA(()),
    ]
    return kernel, scratch


def _run(A_x, A_c_kv, A_w_q, A_w_uk, A_w_uv, A_w_o, B_w1, B_w2, c, w_mod, S=4, **kw):
    B, Sq, M = A_x.shape
    _, Sk, Dc = A_c_kv.shape
    _, H, D = A_w_q.shape
    F = B_w1.shape[1]
    assert Sq == 1
    kernel, scratch = _build(B, H, Sk, D, M, Dc, F, S, **kw)
    out = pl.pallas_call(
        kernel,
        out_shape=jax.ShapeDtypeStruct((B, M), A_x.dtype),
        in_specs=[pl.BlockSpec(memory_space=pl.ANY)] * 10,
        scratch_shapes=scratch,
        compiler_params=pltpu.CompilerParams(vmem_limit_bytes=100 * 1024 * 1024),
    )(A_x.reshape(B, M), A_c_kv.reshape(B, S, Sk // S, Dc), A_w_q.reshape(S, -1, D),
      A_w_uk.reshape(S, -1, D), A_w_uv.reshape(S, -1, D), A_w_o.reshape(S, -1, M), B_w1, B_w2, c, w_mod)
    return out.reshape(B, Sq, M)


@jax.jit
def pallas_adaLN_cond__compressed_kv_cla__dense_activation_relu__decode_kernel(
    A_x: jax.Array,
    A_c_kv: jax.Array,
    A_w_q: jax.Array,
    A_w_uk: jax.Array,
    A_w_uv: jax.Array,
    A_w_o: jax.Array,
    B_x: jax.Array,
    B_w1: jax.Array,
    B_w2: jax.Array,
    c: jax.Array,
    w_mod: jax.Array,
):
    del B_x
    return _run(A_x, A_c_kv, A_w_q, A_w_uk, A_w_uv, A_w_o, B_w1, B_w2, c, w_mod)
```

```python
import jax
import jax.numpy as jnp
import jax.experimental.pallas as pl
import jax.experimental.pallas.tpu as pltpu

_F32 = jnp.float32
_BF16 = jnp.bfloat16
_NT = (((1,), (1,)), ((), ()))
_PRIO = (1, 1, 1, 0)
_S = 4


def _layernorm(x):
    m = jnp.mean(x, axis=-1, keepdims=True)
    d = x - m
    v = jnp.mean(d * d, axis=-1, keepdims=True)
    return d / jnp.sqrt(v + 1e-5)


def _rows(ref):
    v = ref[...]
    return v.reshape(v.shape[0] * v.shape[1], v.shape[2])


def _split_heads(w_ref, tmp_ref):
    w32 = w_ref.bitcast(jnp.uint32)
    for r in range(4):
        tmp_ref[r] = w32[:, pl.ds(r, w32.shape[1] // 4, stride=4), :]


def _head_pair(tmp_ref, j):
    _, s, rows, d = tmp_ref.shape
    w = tmp_ref[j % 4, :, pl.ds(j // 4, rows // 4, stride=4), :].reshape(s * rows // 4, d)
    lo = pltpu.bitcast(w << 16, _F32).astype(_BF16)
    hi = pltpu.bitcast(w & jnp.uint32(0xFFFF0000), _F32).astype(_BF16)
    return lo, hi


def _stream(copies, lo, hi):
    per_step = sum(src.shape[0] // 2 * (src.shape[2] // cols) for src, _, _, _, cols in copies)
    unroll = max(1, len(_PRIO) // per_step)

    def body(it, carry):
        k = 0
        for u in range(unroll):
            for src, dst, sem, rows, cols in copies:
                r = pl.ds(pl.multiple_of((it * unroll + u) * rows, rows), rows)
                for c in range(0, src.shape[2], cols):
                    for s in range(0, src.shape[0], 2):
                        idx = (pl.ds(s, 2), r, pl.ds(c, cols))
                        pltpu.make_async_copy(src.at[idx], dst.at[idx], sem).start(
                            priority=_PRIO[k % len(_PRIO)])
                        k += 1
        return carry

    jax.lax.fori_loop(lo // unroll, hi // unroll, body, 0)


def _wait(dst, sem):
    pltpu.make_async_copy(dst, dst, sem).wait()


def _build(B, H, Sk, D, M, Dc, F, W2=(384, 256, 128, 128), E1=0):
    HP = H // 2
    NC = Dc // 128
    FH = F // 2
    N2 = len(W2)
    O2 = [sum(W2[:i]) for i in range(N2 + 1)]
    assert HP == 16 and O2[-1] == FH

    def kernel(x_hbm, ckv_hbm, wq_hbm, wuk_hbm, wuv_hbm, wo_hbm, w1_hbm, w2_hbm, c_hbm, wm_hbm,
               o_ref,
               x_v, c_v, ckv_v, wq_v, wuk_v, wuv_v, wo_v, w1_v, w2_v, wma_v, wmb_v,
               tmp_v, qa_v, oc_v, fin_v, last_sem):

        def w2_chunk(i):
            return w2_v.at[:, pl.ds(O2[i], W2[i])]

        def main(sems, ksems, fsems):
            s_c, s_x, s_wma, s_wq, s_wuk, s_wuv, s_wo, s_wmb, s_w1 = (sems.at[i] for i in range(9))
            wma = [(wm_hbm.at[:, :, pl.ds(0, 2 * M)], wma_v, s_wma, 8, 2 * M)]
            wqk = [(wq_hbm, wq_v, s_wq, 64, D), (wuk_hbm, wuk_v, s_wuk, 64, D)]
            wvo = [(wuv_hbm, wuv_v, s_wuv, 64, D), (wo_hbm, wo_v, s_wo, 16, M)]
            wmb = [(wm_hbm.at[:, :, pl.ds(2 * M, 4 * M)], wmb_v, s_wmb, 8, 2 * M)]
            w1 = [(w1_hbm, w1_v, s_w1, 8, FH)]

            def kv(g):
                return [(ckv_hbm.at[b], ckv_v.at[b], ksems.at[b], 16, Dc) for b in (2 * g, 2 * g + 1)]

            pltpu.make_async_copy(c_hbm, c_v, s_c).start()
            pltpu.make_async_copy(x_hbm, x_v, s_x).start()
            _stream(wma, 0, 16)
            _stream(wqk, 0, 64)

            _wait(c_v, s_c)
            cc = c_v[...].astype(_F32)
            sc = (cc * jax.nn.sigmoid(cc)).astype(_BF16)
            _wait(wma_v, s_wma)
            moda = jnp.dot(sc, _rows(wma_v), preferred_element_type=_F32)
            _wait(x_v, s_x)
            x = x_v[...].astype(_F32)
            h = (_layernorm(x) * (1.0 + moda[:, M:]) + moda[:, :M]).astype(_BF16)

            _stream(kv(0), 0, 32)
            _wait(wq_v, s_wq)
            _split_heads(wq_v, tmp_v)
            qs = []
            for j in range(HP):
                for w in _head_pair(tmp_v, j):
                    q = jnp.dot(h, w, preferred_element_type=_F32)
                    qs.append((q * D ** -0.5).astype(_BF16))
            _stream(kv(0), 32, 64)
            _wait(wuk_v, s_wuk)
            _split_heads(wuk_v, tmp_v)
            for j in range(HP):
                for s, w in enumerate(_head_pair(tmp_v, j)):
                    qa = jax.lax.dot_general(qs[2 * j + s], w, _NT, preferred_element_type=_F32)
                    for n in range(NC):
                        qa_v[n, pl.ds(2 * j + s, B, stride=H), :] = qa[:, n * 128:(n + 1) * 128]
            _stream(kv(1), 0, 32)

            def attend(b, carry):
                _wait(ckv_v.at[b], ksems.at[b])
                row = pl.ds(pl.multiple_of(b * H, H), H)
                qa = jnp.concatenate([qa_v[n, row, :] for n in range(NC)], axis=1).astype(_BF16)
                s = jax.lax.dot_general(qa, _rows(ckv_v.at[b]), _NT, preferred_element_type=_F32)
                p = jnp.exp(s - jnp.max(s, axis=-1, keepdims=True))
                l = jnp.sum(p, axis=-1, keepdims=True)
                o = jnp.dot(p.astype(_BF16), _rows(ckv_v.at[b]), preferred_element_type=_F32) / l
                for n in range(NC):
                    oc_v[n, row, :] = o[:, n * 128:(n + 1) * 128]

                t = b + 3
                lo = t % 2 * 32

                @pl.when(t < B)
                def _():
                    _stream(kv(t // 2), lo, lo + 32)

                @pl.when(jnp.logical_and(t >= B, t < B + 2))
                def _():
                    _stream(wvo, lo, lo + 32)

                return carry

            jax.lax.fori_loop(0, B, attend, 0)

            _stream(wmb, 0, 16)
            if E1:
                _stream(w1, 0, E1)
            _wait(wuv_v, s_wuv)
            _stream(w1, E1, 16)
            _split_heads(wuv_v, tmp_v)
            _stream(w1, 16, 32)
            ctx = []
            for j in range(HP):
                for s, w in enumerate(_head_pair(tmp_v, j)):
                    oc = jnp.concatenate(
                        [oc_v[n, pl.ds(2 * j + s, B, stride=H), :] for n in range(NC)], axis=1)
                    ctx.append(jnp.dot(oc.astype(_BF16), w, preferred_element_type=_F32).astype(_BF16))
            for i in range(N2):
                sem = fsems.at[i] if i < N2 - 1 else last_sem
                _stream([(w2_hbm, w2_v, sem, 16, M)], O2[i] // 16, O2[i + 1] // 16)
            _wait(wo_v, s_wo)
            att = jnp.dot(jnp.concatenate(ctx, axis=1), _rows(wo_v), preferred_element_type=_F32)
            _wait(wmb_v, s_wmb)
            modb = jnp.dot(sc, _rows(wmb_v), preferred_element_type=_F32)
            x1 = x + modb[:, :M] * att
            h2 = (_layernorm(x1) * (1.0 + modb[:, 2 * M:3 * M]) + modb[:, M:2 * M]).astype(_BF16)

            _wait(w1_v, s_w1)
            a = jnp.maximum(jnp.dot(h2, _rows(w1_v), preferred_element_type=_F32), 0.0)
            a = [jnp.concatenate([a[:, O2[i]:O2[i + 1]], a[:, FH + O2[i]:FH + O2[i + 1]]], axis=1)
                 for i in range(N2)]
            y = jnp.zeros((B, M), _F32)
            for i in range(N2 - 1):
                _wait(w2_chunk(i), fsems.at[i])
                y += jnp.dot(a[i].astype(_BF16), _rows(w2_chunk(i)), preferred_element_type=_F32)
            fin_v[:, :M] = x1
            fin_v[:, M:2 * M] = modb[:, 3 * M:]
            fin_v[:, 2 * M:3 * M] = y
            fin_v[:, 3 * M:] = a[-1]

        pl.run_scoped(main, pltpu.SemaphoreType.DMA((9,)), pltpu.SemaphoreType.DMA((B,)),
                      pltpu.SemaphoreType.DMA((N2 - 1,)))
        x1, gb, y = fin_v[:, :M], fin_v[:, M:2 * M], fin_v[:, 2 * M:3 * M]
        a_last = fin_v[:, 3 * M:].astype(_BF16)
        _wait(w2_chunk(N2 - 1), last_sem)
        y += jnp.dot(a_last, _rows(w2_chunk(N2 - 1)), preferred_element_type=_F32)
        o_ref[...] = (x1 + gb * y).astype(o_ref.dtype)

    scratch = [
        pltpu.VMEM((B, M), _BF16),
        pltpu.VMEM((B, M), _BF16),
        pltpu.VMEM((B, _S, Sk // _S, Dc), _BF16),
        pltpu.VMEM((_S, M * H // _S, D), _BF16),
        pltpu.VMEM((_S, Dc * H // _S, D), _BF16),
        pltpu.VMEM((_S, Dc * H // _S, D), _BF16),
        pltpu.VMEM((_S, H * D // _S, M), _BF16),
        pltpu.VMEM((2, M // 2, F), _BF16),
        pltpu.VMEM((2, FH, M), _BF16),
        pltpu.VMEM((_S, M // _S, 2 * M), _BF16),
        pltpu.VMEM((_S, M // _S, 4 * M), _BF16),
        pltpu.VMEM((4, _S, Dc * HP // _S // 4, D), jnp.uint32),
        pltpu.VMEM((NC, B * H, 128), _F32),
        pltpu.VMEM((NC, B * H, 128), _F32),
        pltpu.VMEM((B, 3 * M + 2 * W2[-1]), _F32),
        pltpu.SemaphoreType.DMA(()),
    ]
    return kernel, scratch


def _run(A_x, A_c_kv, A_w_q, A_w_uk, A_w_uv, A_w_o, B_w1, B_w2, c, w_mod, **kw):
    B, Sq, M = A_x.shape
    _, Sk, Dc = A_c_kv.shape
    _, H, D = A_w_q.shape
    F = B_w1.shape[1]
    assert Sq == 1 and M == Dc
    kernel, scratch = _build(B, H, Sk, D, M, Dc, F, **kw)
    out = pl.pallas_call(
        kernel,
        out_shape=jax.ShapeDtypeStruct((B, M), A_x.dtype),
        in_specs=[pl.BlockSpec(memory_space=pl.ANY)] * 10,
        scratch_shapes=scratch,
        compiler_params=pltpu.CompilerParams(vmem_limit_bytes=100 * 1024 * 1024),
    )(A_x.reshape(B, M), A_c_kv.reshape(B, _S, Sk // _S, Dc), A_w_q.reshape(_S, -1, D),
      A_w_uk.reshape(_S, -1, D), A_w_uv.reshape(_S, -1, D), A_w_o.reshape(_S, -1, M),
      B_w1.reshape(2, -1, F), B_w2.reshape(2, -1, M), c, w_mod.reshape(_S, -1, 6 * M))
    return out.reshape(B, Sq, M)


@jax.jit
def pallas_adaLN_cond__compressed_kv_cla__dense_activation_relu__decode_kernel(
    A_x: jax.Array,
    A_c_kv: jax.Array,
    A_w_q: jax.Array,
    A_w_uk: jax.Array,
    A_w_uv: jax.Array,
    A_w_o: jax.Array,
    B_x: jax.Array,
    B_w1: jax.Array,
    B_w2: jax.Array,
    c: jax.Array,
    w_mod: jax.Array,
):
    del B_x
    return _run(A_x, A_c_kv, A_w_q, A_w_uk, A_w_uv, A_w_o, B_w1, B_w2, c, w_mod)
```

```python
import jax
import jax.numpy as jnp
import jax.experimental.pallas as pl
import jax.experimental.pallas.tpu as pltpu

_F32 = jnp.float32
_BF16 = jnp.bfloat16
_NT = (((1,), (1,)), ((), ()))
_PRIO = (1, 1, 1, 0)
_S = 4


def _layernorm(x):
    m = jnp.mean(x, axis=-1, keepdims=True)
    d = x - m
    v = jnp.mean(d * d, axis=-1, keepdims=True)
    return d / jnp.sqrt(v + 1e-5)


def _rows(ref):
    v = ref[...]
    return v.reshape(v.shape[0] * v.shape[1], v.shape[2])


def _split_heads(w_ref, tmp_ref):
    w32 = w_ref.bitcast(jnp.uint32)
    for r in range(4):
        tmp_ref[r] = w32[:, pl.ds(r, w32.shape[1] // 4, stride=4), :]


def _head_pair(tmp_ref, j):
    _, s, rows, d = tmp_ref.shape
    w = tmp_ref[j % 4, :, pl.ds(j // 4, rows // 4, stride=4), :].reshape(s * rows // 4, d)
    lo = pltpu.bitcast(w << 16, _F32).astype(_BF16)
    hi = pltpu.bitcast(w & jnp.uint32(0xFFFF0000), _F32).astype(_BF16)
    return lo, hi


def _stream(copies, lo, hi, prio=_PRIO):
    per_step = sum(src.shape[0] // 2 * (src.shape[2] // cols) for src, _, _, _, cols in copies)
    unroll = max(1, len(_PRIO) // per_step)

    def body(it, carry):
        k = 0
        for u in range(unroll):
            for src, dst, sem, rows, cols in copies:
                r = pl.ds(pl.multiple_of((it * unroll + u) * rows, rows), rows)
                for c in range(0, src.shape[2], cols):
                    for s in range(0, src.shape[0], 2):
                        idx = (pl.ds(s, 2), r, pl.ds(c, cols))
                        pltpu.make_async_copy(src.at[idx], dst.at[idx], sem).start(
                            priority=prio[k % len(prio)])
                        k += 1
        return carry

    jax.lax.fori_loop(lo // unroll, hi // unroll, body, 0)


def _wait(dst, sem):
    pltpu.make_async_copy(dst, dst, sem).wait()


def _build(B, H, Sk, D, M, Dc, F, W2=(256, 256, 128, 128, 128), p2=(_PRIO,) * 5, p1=_PRIO):
    HP = H // 2
    NC = Dc // 128
    FH = F // 2
    N2 = len(W2)
    O2 = [sum(W2[:i]) for i in range(N2 + 1)]
    assert HP == 16 and O2[-1] == FH

    def kernel(x_hbm, ckv_hbm, wq_hbm, wuk_hbm, wuv_hbm, wo_hbm, w1_hbm, w2_hbm, c_hbm, wm_hbm,
               o_ref,
               x_v, c_v, ckv_v, wq_v, wuk_v, wuv_v, wo_v, w1_v, w2_v, wma_v, wmb_v,
               tmp_v, qa_v, oc_v):

        def main(sems, ksems, fsems):
            s_c, s_x, s_wma, s_wq, s_wuk, s_wuv, s_wo, s_wmb, s_w1 = (sems.at[i] for i in range(9))
            wma = [(wm_hbm.at[:, :, pl.ds(0, 2 * M)], wma_v, s_wma, 8, 2 * M)]
            wqk = [(wq_hbm, wq_v, s_wq, 64, D), (wuk_hbm, wuk_v, s_wuk, 64, D)]
            wvo = [(wuv_hbm, wuv_v, s_wuv, 64, D), (wo_hbm, wo_v, s_wo, 16, M)]
            wmb = [(wm_hbm.at[:, :, pl.ds(2 * M, 4 * M)], wmb_v, s_wmb, 8, 2 * M)]
            w1 = [(w1_hbm, w1_v, s_w1, 8, FH)]

            def kv(g):
                return [(ckv_hbm.at[b], ckv_v.at[b], ksems.at[b], 16, Dc) for b in (2 * g, 2 * g + 1)]

            pltpu.make_async_copy(c_hbm, c_v, s_c).start()
            pltpu.make_async_copy(x_hbm, x_v, s_x).start()
            _stream(wma, 0, 16)
            _stream(wqk, 0, 64)

            _wait(c_v, s_c)
            cc = c_v[...].astype(_F32)
            sc = (cc * jax.nn.sigmoid(cc)).astype(_BF16)
            _wait(wma_v, s_wma)
            moda = jnp.dot(sc, _rows(wma_v), preferred_element_type=_F32)
            _wait(x_v, s_x)
            x = x_v[...].astype(_F32)
            h = (_layernorm(x) * (1.0 + moda[:, M:]) + moda[:, :M]).astype(_BF16)

            _stream(kv(0), 0, 32)
            _wait(wq_v, s_wq)
            _split_heads(wq_v, tmp_v)
            qs = []
            for j in range(HP):
                for w in _head_pair(tmp_v, j):
                    q = jnp.dot(h, w, preferred_element_type=_F32)
                    qs.append((q * D ** -0.5).astype(_BF16))
            _stream(kv(0), 32, 64)
            _wait(wuk_v, s_wuk)
            _split_heads(wuk_v, tmp_v)
            for j in range(HP):
                for s, w in enumerate(_head_pair(tmp_v, j)):
                    qa = jax.lax.dot_general(qs[2 * j + s], w, _NT, preferred_element_type=_F32)
                    for n in range(NC):
                        qa_v[n, pl.ds(2 * j + s, B, stride=H), :] = qa[:, n * 128:(n + 1) * 128]
            _stream(kv(1), 0, 32)

            def attend(b, carry):
                _wait(ckv_v.at[b], ksems.at[b])
                row = pl.ds(pl.multiple_of(b * H, H), H)
                qa = jnp.concatenate([qa_v[n, row, :] for n in range(NC)], axis=1).astype(_BF16)
                s = jax.lax.dot_general(qa, _rows(ckv_v.at[b]), _NT, preferred_element_type=_F32)
                p = jnp.exp(s - jnp.max(s, axis=-1, keepdims=True))
                l = jnp.sum(p, axis=-1, keepdims=True)
                o = jnp.dot(p.astype(_BF16), _rows(ckv_v.at[b]), preferred_element_type=_F32) / l
                for n in range(NC):
                    oc_v[n, row, :] = o[:, n * 128:(n + 1) * 128]

                t = b + 3
                lo = t % 2 * 32

                @pl.when(t < B)
                def _():
                    _stream(kv(t // 2), lo, lo + 32)

                @pl.when(jnp.logical_and(t >= B, t < B + 2))
                def _():
                    _stream(wvo, lo, lo + 32)

                return carry

            jax.lax.fori_loop(0, B, attend, 0)

            _stream(wmb, 0, 16)
            _stream(w1, 0, 16, p1)
            _wait(wuv_v, s_wuv)
            _split_heads(wuv_v, tmp_v)
            _stream(w1, 16, 32, p1)
            ctx = []
            for j in range(HP):
                for s, w in enumerate(_head_pair(tmp_v, j)):
                    oc = jnp.concatenate(
                        [oc_v[n, pl.ds(2 * j + s, B, stride=H), :] for n in range(NC)], axis=1)
                    ctx.append(jnp.dot(oc.astype(_BF16), w, preferred_element_type=_F32).astype(_BF16))
            for i in range(N2):
                _stream([(w2_hbm, w2_v, fsems.at[i], 16, M)], O2[i] // 16, O2[i + 1] // 16, p2[i])
            _wait(wo_v, s_wo)
            att = jnp.dot(jnp.concatenate(ctx, axis=1), _rows(wo_v), preferred_element_type=_F32)
            _wait(wmb_v, s_wmb)
            modb = jnp.dot(sc, _rows(wmb_v), preferred_element_type=_F32)
            x1 = x + modb[:, :M] * att
            h2 = (_layernorm(x1) * (1.0 + modb[:, 2 * M:3 * M]) + modb[:, M:2 * M]).astype(_BF16)

            _wait(w1_v, s_w1)
            a = jnp.maximum(jnp.dot(h2, _rows(w1_v), preferred_element_type=_F32), 0.0)
            a = a.astype(_BF16)
            y = jnp.zeros((B, M), _F32)
            for i in range(N2):
                chunk = w2_v.at[:, pl.ds(O2[i], W2[i])]
                a_i = jnp.concatenate([a[:, O2[i]:O2[i + 1]], a[:, FH + O2[i]:FH + O2[i + 1]]], axis=1)
                _wait(chunk, fsems.at[i])
                y += jnp.dot(a_i, _rows(chunk), preferred_element_type=_F32)
            o_ref[...] = (x1 + modb[:, 3 * M:] * y).astype(o_ref.dtype)

        pl.run_scoped(main, pltpu.SemaphoreType.DMA((9,)), pltpu.SemaphoreType.DMA((B,)),
                      pltpu.SemaphoreType.DMA((N2,)))

    scratch = [
        pltpu.VMEM((B, M), _BF16),
        pltpu.VMEM((B, M), _BF16),
        pltpu.VMEM((B, _S, Sk // _S, Dc), _BF16),
        pltpu.VMEM((_S, M * H // _S, D), _BF16),
        pltpu.VMEM((_S, Dc * H // _S, D), _BF16),
        pltpu.VMEM((_S, Dc * H // _S, D), _BF16),
        pltpu.VMEM((_S, H * D // _S, M), _BF16),
        pltpu.VMEM((2, M // 2, F), _BF16),
        pltpu.VMEM((2, FH, M), _BF16),
        pltpu.VMEM((_S, M // _S, 2 * M), _BF16),
        pltpu.VMEM((_S, M // _S, 4 * M), _BF16),
        pltpu.VMEM((4, _S, Dc * HP // _S // 4, D), jnp.uint32),
        pltpu.VMEM((NC, B * H, 128), _F32),
        pltpu.VMEM((NC, B * H, 128), _F32),
    ]
    return kernel, scratch


def _run(A_x, A_c_kv, A_w_q, A_w_uk, A_w_uv, A_w_o, B_w1, B_w2, c, w_mod, **kw):
    B, Sq, M = A_x.shape
    _, Sk, Dc = A_c_kv.shape
    _, H, D = A_w_q.shape
    F = B_w1.shape[1]
    assert Sq == 1 and M == Dc
    kernel, scratch = _build(B, H, Sk, D, M, Dc, F, **kw)
    out = pl.pallas_call(
        kernel,
        out_shape=jax.ShapeDtypeStruct((B, M), A_x.dtype),
        in_specs=[pl.BlockSpec(memory_space=pl.ANY)] * 10,
        scratch_shapes=scratch,
        compiler_params=pltpu.CompilerParams(vmem_limit_bytes=100 * 1024 * 1024),
    )(A_x.reshape(B, M), A_c_kv.reshape(B, _S, Sk // _S, Dc), A_w_q.reshape(_S, -1, D),
      A_w_uk.reshape(_S, -1, D), A_w_uv.reshape(_S, -1, D), A_w_o.reshape(_S, -1, M),
      B_w1.reshape(2, -1, F), B_w2.reshape(2, -1, M), c, w_mod.reshape(_S, -1, 6 * M))
    return out.reshape(B, Sq, M)


@jax.jit
def pallas_adaLN_cond__compressed_kv_cla__dense_activation_relu__decode_kernel(
    A_x: jax.Array,
    A_c_kv: jax.Array,
    A_w_q: jax.Array,
    A_w_uk: jax.Array,
    A_w_uv: jax.Array,
    A_w_o: jax.Array,
    B_x: jax.Array,
    B_w1: jax.Array,
    B_w2: jax.Array,
    c: jax.Array,
    w_mod: jax.Array,
):
    del B_x
    return _run(A_x, A_c_kv, A_w_q, A_w_uk, A_w_uv, A_w_o, B_w1, B_w2, c, w_mod)
```

```python
import functools

import jax
import jax.numpy as jnp
import jax.experimental.pallas as pl
import jax.experimental.pallas.tpu as pltpu

_F32 = jnp.float32
_BF16 = jnp.bfloat16
_NT = (((1,), (1,)), ((), ()))
_PRIO = (1, 1, 1, 0)
_S = 4


def _layernorm(x):
    m = jnp.mean(x, axis=-1, keepdims=True)
    d = x - m
    v = jnp.mean(d * d, axis=-1, keepdims=True)
    return d / jnp.sqrt(v + 1e-5)


def _rows(ref):
    v = ref[...]
    return v.reshape(v.shape[0] * v.shape[1], v.shape[2])


def _split_heads(w_ref, tmp_ref):
    w32 = w_ref.bitcast(jnp.uint32)
    for r in range(4):
        tmp_ref[r] = w32[:, pl.ds(r, w32.shape[1] // 4, stride=4), :]


def _head_pair(tmp_ref, j):
    _, s, rows, d = tmp_ref.shape
    w = tmp_ref[j % 4, :, pl.ds(j // 4, rows // 4, stride=4), :].reshape(s * rows // 4, d)
    lo = pltpu.bitcast(w << 16, _F32).astype(_BF16)
    hi = pltpu.bitcast(w & jnp.uint32(0xFFFF0000), _F32).astype(_BF16)
    return lo, hi


def _stream(copies, lo, hi):
    per_step = sum(src.shape[0] // 2 * (src.shape[2] // cols) for src, _, _, _, cols in copies)
    unroll = max(1, len(_PRIO) // per_step)

    def body(it, carry):
        k = 0
        for u in range(unroll):
            for src, dst, sem, rows, cols in copies:
                r = pl.ds(pl.multiple_of((it * unroll + u) * rows, rows), rows)
                for c in range(0, src.shape[2], cols):
                    for s in range(0, src.shape[0], 2):
                        idx = (pl.ds(s, 2), r, pl.ds(c, cols))
                        pltpu.make_async_copy(src.at[idx], dst.at[idx], sem).start(
                            priority=_PRIO[k % len(_PRIO)])
                        k += 1
        return carry

    jax.lax.fori_loop(lo // unroll, hi // unroll, body, 0)


def _wait(dst, sem):
    pltpu.make_async_copy(dst, dst, sem).wait()


def _build(B, H, Sk, D, M, Dc, F, W2=(256, 256, 128, 128, 128), V1=32, V2=48, E1=16):
    HP = H // 2
    NC = Dc // 128
    FH = F // 2
    N2 = len(W2)
    O2 = [sum(W2[:i]) for i in range(N2 + 1)]
    assert B == 8 and HP == 16 and O2[-1] == FH

    def kernel(x_hbm, ckv_hbm, wq_hbm, wuk_hbm, wuv_hbm, wo_hbm, w1_hbm, w2_hbm, c_hbm, wm_hbm,
               o_ref,
               x_v, c_v, ckv_v, wq_v, wuk_v, wuv_v, wo_v, w1_v, w2_v, wma_v, wmb_v,
               tmp_v, qa_v, oc_v):

        def main(sems, ksems, fsems):
            s_c, s_x, s_wma, s_wq, s_wuk, s_wuv, s_wo, s_wmb, s_w1 = (sems.at[i] for i in range(9))
            wma = [(wm_hbm.at[:, :, pl.ds(0, 2 * M)], wma_v, s_wma, 8, 2 * M)]
            wqk = [(wq_hbm, wq_v, s_wq, 64, D), (wuk_hbm, wuk_v, s_wuk, 64, D)]
            wvo = [(wuv_hbm, wuv_v, s_wuv, 64, D), (wo_hbm, wo_v, s_wo, 16, M)]
            wmb = [(wm_hbm.at[:, :, pl.ds(2 * M, 4 * M)], wmb_v, s_wmb, 8, 2 * M)]
            w1 = [(w1_hbm, w1_v, s_w1, 8, FH)]
            kv = [(ckv_hbm.at[b], ckv_v.at[b], ksems.at[b], 16, Dc) for b in range(B)]
            kva, kvb = kv[:B // 2], kv[B // 2:]

            pltpu.make_async_copy(c_hbm, c_v, s_c).start()
            pltpu.make_async_copy(x_hbm, x_v, s_x).start()
            _stream(wma, 0, 16)
            _stream(wqk, 0, 64)

            _wait(c_v, s_c)
            cc = c_v[...].astype(_F32)
            sc = (cc * jax.nn.sigmoid(cc)).astype(_BF16)
            _wait(wma_v, s_wma)
            moda = jnp.dot(sc, _rows(wma_v), preferred_element_type=_F32)
            _wait(x_v, s_x)
            x = x_v[...].astype(_F32)
            h = (_layernorm(x) * (1.0 + moda[:, M:]) + moda[:, :M]).astype(_BF16)

            _stream(kva, 0, 16)
            _wait(wq_v, s_wq)
            _split_heads(wq_v, tmp_v)
            qs = []
            for j in range(HP):
                for w in _head_pair(tmp_v, j):
                    q = jnp.dot(h, w, preferred_element_type=_F32)
                    qs.append((q * D ** -0.5).astype(_BF16))
            _stream(kva, 16, 32)
            _wait(wuk_v, s_wuk)
            _split_heads(wuk_v, tmp_v)
            for j in range(HP):
                for s, w in enumerate(_head_pair(tmp_v, j)):
                    qa = jax.lax.dot_general(qs[2 * j + s], w, _NT, preferred_element_type=_F32)
                    for n in range(NC):
                        qa_v[n, pl.ds(2 * j + s, B, stride=H), :] = qa[:, n * 128:(n + 1) * 128]
            _stream(kva, 32, 64)
            _stream(kvb, 0, 16)

            ahead = [(kvb, 16, 32), (kvb, 32, 48), (kvb, 48, 64),
                     (wvo, 0, V1), (wvo, V1, V2), (wvo, V2, 64), (wmb, 0, 16)]

            def attend(b, carry):
                _wait(ckv_v.at[b], ksems.at[b])
                row = pl.ds(pl.multiple_of(b * H, H), H)
                qa = jnp.concatenate([qa_v[n, row, :] for n in range(NC)], axis=1).astype(_BF16)
                s = jax.lax.dot_general(qa, _rows(ckv_v.at[b]), _NT, preferred_element_type=_F32)
                p = jnp.exp(s - jnp.max(s, axis=-1, keepdims=True))
                l = jnp.sum(p, axis=-1, keepdims=True)
                o = jnp.dot(p.astype(_BF16), _rows(ckv_v.at[b]), preferred_element_type=_F32) / l
                for n in range(NC):
                    oc_v[n, row, :] = o[:, n * 128:(n + 1) * 128]

                for k, request in enumerate(ahead):
                    pl.when(b == k)(functools.partial(_stream, *request))
                return carry

            jax.lax.fori_loop(0, B, attend, 0)

            _stream(w1, 0, E1)
            _wait(wuv_v, s_wuv)
            _split_heads(wuv_v, tmp_v)
            _stream(w1, E1, 32)
            ctx = []
            for j in range(HP):
                for s, w in enumerate(_head_pair(tmp_v, j)):
                    oc = jnp.concatenate(
                        [oc_v[n, pl.ds(2 * j + s, B, stride=H), :] for n in range(NC)], axis=1)
                    ctx.append(jnp.dot(oc.astype(_BF16), w, preferred_element_type=_F32).astype(_BF16))
            for i in range(N2):
                _stream([(w2_hbm, w2_v, fsems.at[i], 16, M)], O2[i] // 16, O2[i + 1] // 16)
            _wait(wo_v, s_wo)
            att = jnp.dot(jnp.concatenate(ctx, axis=1), _rows(wo_v), preferred_element_type=_F32)
            _wait(wmb_v, s_wmb)
            modb = jnp.dot(sc, _rows(wmb_v), preferred_element_type=_F32)
            x1 = x + modb[:, :M] * att
            h2 = (_layernorm(x1) * (1.0 + modb[:, 2 * M:3 * M]) + modb[:, M:2 * M]).astype(_BF16)

            _wait(w1_v, s_w1)
            a = jnp.maximum(jnp.dot(h2, _rows(w1_v), preferred_element_type=_F32), 0.0)
            a = a.astype(_BF16)
            y = jnp.zeros((B, M), _F32)
            for i in range(N2):
                chunk = w2_v.at[:, pl.ds(O2[i], W2[i])]
                a_i = jnp.concatenate([a[:, O2[i]:O2[i + 1]], a[:, FH + O2[i]:FH + O2[i + 1]]], axis=1)
                _wait(chunk, fsems.at[i])
                y += jnp.dot(a_i, _rows(chunk), preferred_element_type=_F32)
            o_ref[...] = (x1 + modb[:, 3 * M:] * y).astype(o_ref.dtype)

        pl.run_scoped(main, pltpu.SemaphoreType.DMA((9,)), pltpu.SemaphoreType.DMA((B,)),
                      pltpu.SemaphoreType.DMA((N2,)))

    scratch = [
        pltpu.VMEM((B, M), _BF16),
        pltpu.VMEM((B, M), _BF16),
        pltpu.VMEM((B, _S, Sk // _S, Dc), _BF16),
        pltpu.VMEM((_S, M * H // _S, D), _BF16),
        pltpu.VMEM((_S, Dc * H // _S, D), _BF16),
        pltpu.VMEM((_S, Dc * H // _S, D), _BF16),
        pltpu.VMEM((_S, H * D // _S, M), _BF16),
        pltpu.VMEM((2, M // 2, F), _BF16),
        pltpu.VMEM((2, FH, M), _BF16),
        pltpu.VMEM((_S, M // _S, 2 * M), _BF16),
        pltpu.VMEM((_S, M // _S, 4 * M), _BF16),
        pltpu.VMEM((4, _S, Dc * HP // _S // 4, D), jnp.uint32),
        pltpu.VMEM((NC, B * H, 128), _F32),
        pltpu.VMEM((NC, B * H, 128), _F32),
    ]
    return kernel, scratch


def _run(A_x, A_c_kv, A_w_q, A_w_uk, A_w_uv, A_w_o, B_w1, B_w2, c, w_mod, **kw):
    B, Sq, M = A_x.shape
    _, Sk, Dc = A_c_kv.shape
    _, H, D = A_w_q.shape
    F = B_w1.shape[1]
    assert Sq == 1 and M == Dc
    kernel, scratch = _build(B, H, Sk, D, M, Dc, F, **kw)
    out = pl.pallas_call(
        kernel,
        out_shape=jax.ShapeDtypeStruct((B, M), A_x.dtype),
        in_specs=[pl.BlockSpec(memory_space=pl.ANY)] * 10,
        scratch_shapes=scratch,
        compiler_params=pltpu.CompilerParams(vmem_limit_bytes=100 * 1024 * 1024),
    )(A_x.reshape(B, M), A_c_kv.reshape(B, _S, Sk // _S, Dc), A_w_q.reshape(_S, -1, D),
      A_w_uk.reshape(_S, -1, D), A_w_uv.reshape(_S, -1, D), A_w_o.reshape(_S, -1, M),
      B_w1.reshape(2, -1, F), B_w2.reshape(2, -1, M), c, w_mod.reshape(_S, -1, 6 * M))
    return out.reshape(B, Sq, M)


@jax.jit
def pallas_adaLN_cond__compressed_kv_cla__dense_activation_relu__decode_kernel(
    A_x: jax.Array,
    A_c_kv: jax.Array,
    A_w_q: jax.Array,
    A_w_uk: jax.Array,
    A_w_uv: jax.Array,
    A_w_o: jax.Array,
    B_x: jax.Array,
    B_w1: jax.Array,
    B_w2: jax.Array,
    c: jax.Array,
    w_mod: jax.Array,
):
    del B_x
    return _run(A_x, A_c_kv, A_w_q, A_w_uk, A_w_uv, A_w_o, B_w1, B_w2, c, w_mod)
```

```python
import functools

import jax
import jax.numpy as jnp
import jax.experimental.pallas as pl
import jax.experimental.pallas.tpu as pltpu
import numpy as np

_F32 = jnp.float32
_BF16 = jnp.bfloat16
_NT = (((1,), (1,)), ((), ()))
_PRIO = (1, 1, 1, 0)
_S = 4


def _layernorm(x):
    m = jnp.mean(x, axis=-1, keepdims=True)
    d = x - m
    v = jnp.mean(d * d, axis=-1, keepdims=True)
    return d / jnp.sqrt(v + 1e-5)


def _rows(ref):
    v = ref[...]
    return v.reshape(v.shape[0] * v.shape[1], v.shape[2])


def _split_heads(w_ref, tmp_ref):
    w32 = w_ref.bitcast(jnp.uint32)
    for r in range(4):
        tmp_ref[r] = w32[:, pl.ds(r, w32.shape[1] // 4, stride=4), :]


def _head_pair(tmp_ref, j):
    _, s, rows, d = tmp_ref.shape
    w = tmp_ref[j % 4, :, pl.ds(j // 4, rows // 4, stride=4), :].reshape(s * rows // 4, d)
    lo = pltpu.bitcast(w << 16, _F32).astype(_BF16)
    hi = pltpu.bitcast(w & np.uint32(0xFFFF0000), _F32).astype(_BF16)
    return lo, hi


def _stream(copies, lo, hi):
    per_step = sum(src.shape[0] // 2 * (src.shape[2] // cols) for src, _, _, _, cols in copies)
    unroll = max(1, len(_PRIO) // per_step)

    def body(it, carry):
        k = 0
        for u in range(unroll):
            for src, dst, sem, rows, cols in copies:
                r = pl.ds(pl.multiple_of((it * unroll + u) * rows, rows), rows)
                for c in range(0, src.shape[2], cols):
                    for s in range(0, src.shape[0], 2):
                        idx = (pl.ds(s, 2), r, pl.ds(c, cols))
                        pltpu.make_async_copy(src.at[idx], dst.at[idx], sem).start(
                            priority=_PRIO[k % len(_PRIO)])
                        k += 1
        return carry

    jax.lax.fori_loop(lo // unroll, hi // unroll, body, 0)


def _wait(dst, sem):
    pltpu.make_async_copy(dst, dst, sem).wait()


def _build(B, H, Sk, D, M, Dc, F):
    HP = H // 2
    NC = Dc // 128
    FH = F // 2
    W2 = (256, 256, 128, 128, 128)
    N2 = len(W2)
    O2 = [sum(W2[:i]) for i in range(N2 + 1)]
    assert (B, H, Sk, D, M, Dc, FH) == (8, 32, 4096, 128, 512, 512, O2[-1])

    def kernel(x_hbm, ckv_hbm, wq_hbm, wuk_hbm, wuv_hbm, wo_hbm, w1_hbm, w2_hbm, c_hbm, wm_hbm,
               o_ref,
               x_v, c_v, ckv_v, wq_v, wuk_v, wuv_v, wo_v, w1_v, w2_v, wma_v, wmb_v,
               tmp_v, qa_v, oc_v):

        def main(sems, ksems, fsems):
            s_c, s_x, s_wma, s_wq, s_wuk, s_wuv, s_wo, s_wmb, s_w1 = (sems.at[i] for i in range(9))
            wma = [(wm_hbm.at[:, :, pl.ds(0, 2 * M)], wma_v, s_wma, 8, 2 * M)]
            wqk = [(wq_hbm, wq_v, s_wq, 64, D), (wuk_hbm, wuk_v, s_wuk, 64, D)]
            wvo = [(wuv_hbm, wuv_v, s_wuv, 64, D), (wo_hbm, wo_v, s_wo, 16, M)]
            wmb = [(wm_hbm.at[:, :, pl.ds(2 * M, 4 * M)], wmb_v, s_wmb, 8, 2 * M)]
            w1 = [(w1_hbm, w1_v, s_w1, 8, FH)]
            kv = [(ckv_hbm.at[b], ckv_v.at[b], ksems.at[b], 16, Dc) for b in range(B)]
            kva, kvb = kv[:B // 2], kv[B // 2:]

            pltpu.make_async_copy(c_hbm, c_v, s_c).start()
            pltpu.make_async_copy(x_hbm, x_v, s_x).start()
            _stream(wma, 0, 16)
            _stream(wqk, 0, 64)

            _wait(c_v, s_c)
            cc = c_v[...].astype(_F32)
            sc = (cc * jax.nn.sigmoid(cc)).astype(_BF16)
            _wait(wma_v, s_wma)
            moda = jnp.dot(sc, _rows(wma_v), preferred_element_type=_F32)
            _wait(x_v, s_x)
            x = x_v[...].astype(_F32)
            h = (_layernorm(x) * (1.0 + moda[:, M:]) + moda[:, :M]).astype(_BF16)

            _stream(kva, 0, 16)
            _wait(wq_v, s_wq)
            _split_heads(wq_v, tmp_v)
            qs = []
            for j in range(HP):
                for w in _head_pair(tmp_v, j):
                    q = jnp.dot(h, w, preferred_element_type=_F32)
                    qs.append((q * D ** -0.5).astype(_BF16))
            _stream(kva, 16, 32)
            _wait(wuk_v, s_wuk)
            _split_heads(wuk_v, tmp_v)
            for j in range(HP):
                for s, w in enumerate(_head_pair(tmp_v, j)):
                    qa = jax.lax.dot_general(qs[2 * j + s], w, _NT, preferred_element_type=_F32)
                    for n in range(NC):
                        qa_v[n, pl.ds(2 * j + s, B, stride=H), :] = qa[:, n * 128:(n + 1) * 128]
            _stream(kva, 32, 64)
            _stream(kvb, 0, 16)

            ahead = [(kvb, 16, 32), (kvb, 32, 48), (kvb, 48, 64),
                     (wvo, 0, 32), (wvo, 32, 48), (wvo, 48, 64), (wmb, 0, 16)]

            def attend(b, carry):
                _wait(ckv_v.at[b], ksems.at[b])
                row = pl.ds(pl.multiple_of(b * H, H), H)
                qa = jnp.concatenate([qa_v[n, row, :] for n in range(NC)], axis=1).astype(_BF16)
                s = jax.lax.dot_general(qa, _rows(ckv_v.at[b]), _NT, preferred_element_type=_F32)
                p = jnp.exp(s - jnp.max(s, axis=-1, keepdims=True))
                l = jnp.sum(p, axis=-1, keepdims=True)
                o = jnp.dot(p.astype(_BF16), _rows(ckv_v.at[b]), preferred_element_type=_F32) / l
                for n in range(NC):
                    oc_v[n, row, :] = o[:, n * 128:(n + 1) * 128]

                for k, request in enumerate(ahead):
                    pl.when(b == k)(functools.partial(_stream, *request))
                return carry

            jax.lax.fori_loop(0, B, attend, 0)

            _stream(w1, 0, 16)
            _wait(wuv_v, s_wuv)
            _split_heads(wuv_v, tmp_v)
            _stream(w1, 16, 32)
            ctx = []
            for j in range(HP):
                for s, w in enumerate(_head_pair(tmp_v, j)):
                    oc = jnp.concatenate(
                        [oc_v[n, pl.ds(2 * j + s, B, stride=H), :] for n in range(NC)], axis=1)
                    ctx.append(jnp.dot(oc.astype(_BF16), w, preferred_element_type=_F32).astype(_BF16))
            for i in range(N2):
                _stream([(w2_hbm, w2_v, fsems.at[i], 16, M)], O2[i] // 16, O2[i + 1] // 16)
            _wait(wo_v, s_wo)
            att = jnp.dot(jnp.concatenate(ctx, axis=1), _rows(wo_v), preferred_element_type=_F32)
            _wait(wmb_v, s_wmb)
            modb = jnp.dot(sc, _rows(wmb_v), preferred_element_type=_F32)
            x1 = x + modb[:, :M] * att
            h2 = (_layernorm(x1) * (1.0 + modb[:, 2 * M:3 * M]) + modb[:, M:2 * M]).astype(_BF16)

            _wait(w1_v, s_w1)
            a = jnp.maximum(jnp.dot(h2, _rows(w1_v), preferred_element_type=_F32), 0.0).astype(_BF16)
            y = jnp.zeros((B, M), _F32)
            for i in range(N2):
                chunk = w2_v.at[:, pl.ds(O2[i], W2[i])]
                a_i = jnp.concatenate([a[:, O2[i]:O2[i + 1]], a[:, FH + O2[i]:FH + O2[i + 1]]], axis=1)
                _wait(chunk, fsems.at[i])
                y += jnp.dot(a_i, _rows(chunk), preferred_element_type=_F32)
            o_ref[...] = (x1 + modb[:, 3 * M:] * y).astype(o_ref.dtype)

        pl.run_scoped(main, pltpu.SemaphoreType.DMA((9,)), pltpu.SemaphoreType.DMA((B,)),
                      pltpu.SemaphoreType.DMA((N2,)))

    scratch = [
        pltpu.VMEM((B, M), _BF16),
        pltpu.VMEM((B, M), _BF16),
        pltpu.VMEM((B, _S, Sk // _S, Dc), _BF16),
        pltpu.VMEM((_S, M * H // _S, D), _BF16),
        pltpu.VMEM((_S, Dc * H // _S, D), _BF16),
        pltpu.VMEM((_S, Dc * H // _S, D), _BF16),
        pltpu.VMEM((_S, H * D // _S, M), _BF16),
        pltpu.VMEM((2, M // 2, F), _BF16),
        pltpu.VMEM((2, FH, M), _BF16),
        pltpu.VMEM((_S, M // _S, 2 * M), _BF16),
        pltpu.VMEM((_S, M // _S, 4 * M), _BF16),
        pltpu.VMEM((4, _S, Dc * HP // _S // 4, D), jnp.uint32),
        pltpu.VMEM((NC, B * H, 128), _F32),
        pltpu.VMEM((NC, B * H, 128), _F32),
    ]
    return kernel, scratch


@jax.jit
def pallas_adaLN_cond__compressed_kv_cla__dense_activation_relu__decode_kernel(
    A_x: jax.Array,
    A_c_kv: jax.Array,
    A_w_q: jax.Array,
    A_w_uk: jax.Array,
    A_w_uv: jax.Array,
    A_w_o: jax.Array,
    B_x: jax.Array,
    B_w1: jax.Array,
    B_w2: jax.Array,
    c: jax.Array,
    w_mod: jax.Array,
):
    del B_x
    B, Sq, M = A_x.shape
    _, Sk, Dc = A_c_kv.shape
    _, H, D = A_w_q.shape
    F = B_w1.shape[1]
    assert Sq == 1
    kernel, scratch = _build(B, H, Sk, D, M, Dc, F)
    out = pl.pallas_call(
        kernel,
        out_shape=jax.ShapeDtypeStruct((B, M), A_x.dtype),
        in_specs=[pl.BlockSpec(memory_space=pl.ANY)] * 10,
        scratch_shapes=scratch,
        compiler_params=pltpu.CompilerParams(vmem_limit_bytes=100 * 1024 * 1024),
    )(A_x.reshape(B, M), A_c_kv.reshape(B, _S, Sk // _S, Dc), A_w_q.reshape(_S, -1, D),
      A_w_uk.reshape(_S, -1, D), A_w_uv.reshape(_S, -1, D), A_w_o.reshape(_S, -1, M),
      B_w1.reshape(2, -1, F), B_w2.reshape(2, -1, M), c, w_mod.reshape(_S, -1, 6 * M))
    return out.reshape(B, Sq, M)
```

```python
import functools

import jax
import jax.numpy as jnp
import jax.experimental.pallas as pl
import jax.experimental.pallas.tpu as pltpu
import numpy as np

_F32 = jnp.float32
_BF16 = jnp.bfloat16
_NT = (((1,), (1,)), ((), ()))
_PRIO = (1, 1, 1, 0)
_S = 4


def _layernorm(x):
    m = jnp.mean(x, axis=-1, keepdims=True)
    d = x - m
    v = jnp.mean(d * d, axis=-1, keepdims=True)
    return d / jnp.sqrt(v + 1e-5)


def _rows(ref):
    v = ref[...]
    return v.reshape(v.shape[0] * v.shape[1], v.shape[2])


def _split_heads(w_ref, w32_ref, tmp_ref):
    w32_ref[...] = pltpu.bitcast(w_ref[...], jnp.uint32)
    for r in range(4):
        tmp_ref[r] = w32_ref[:, pl.ds(r, w32_ref.shape[1] // 4, stride=4), :]


def _head_pair(tmp_ref, j):
    _, s, rows, d = tmp_ref.shape
    w = tmp_ref[j % 4, :, pl.ds(j // 4, rows // 4, stride=4), :].reshape(s * rows // 4, d)
    lo = pltpu.bitcast(w << 16, _F32).astype(_BF16)
    hi = pltpu.bitcast(w & np.uint32(0xFFFF0000), _F32).astype(_BF16)
    return lo, hi


def _stream(copies, lo, hi):
    per_step = sum(src.shape[0] // 2 * (src.shape[2] // cols) for src, _, _, _, cols in copies)
    unroll = max(1, len(_PRIO) // per_step)

    def body(it, carry):
        k = 0
        for u in range(unroll):
            for src, dst, sem, rows, cols in copies:
                r = pl.ds(pl.multiple_of((it * unroll + u) * rows, rows), rows)
                for c in range(0, src.shape[2], cols):
                    for s in range(0, src.shape[0], 2):
                        idx = (pl.ds(s, 2), r, pl.ds(c, cols))
                        pltpu.make_async_copy(src.at[idx], dst.at[idx], sem).start(
                            priority=_PRIO[k % len(_PRIO)])
                        k += 1
        return carry

    jax.lax.fori_loop(lo // unroll, hi // unroll, body, 0)


def _wait(dst, sem):
    pltpu.make_async_copy(dst, dst, sem).wait()


def _build(B, H, Sk, D, M, Dc, F):
    HP = H // 2
    NC = Dc // 128
    FH = F // 2
    W2 = (256, 256, 128, 128, 128)
    N2 = len(W2)
    O2 = [sum(W2[:i]) for i in range(N2 + 1)]
    assert (B, H, Sk, D, M, Dc, FH) == (8, 32, 4096, 128, 512, 512, O2[-1])

    def kernel(x_hbm, ckv_hbm, wq_hbm, wuk_hbm, wuv_hbm, wo_hbm, w1_hbm, w2_hbm, c_hbm, wm_hbm,
               o_ref,
               x_v, c_v, ckv_v, wq_v, wuk_v, wuv_v, wo_v, w1_v, w2_v, wma_v, wmb_v,
               w32_v, tmp_v, qa_v, oc_v):

        def main(sems, ksems, fsems):
            s_c, s_x, s_wma, s_wq, s_wuk, s_wuv, s_wo, s_wmb, s_w1 = (sems.at[i] for i in range(9))
            wma = [(wm_hbm.at[:, :, pl.ds(0, 2 * M)], wma_v, s_wma, 8, 2 * M)]
            wqk = [(wq_hbm, wq_v, s_wq, 64, D), (wuk_hbm, wuk_v, s_wuk, 64, D)]
            wvo = [(wuv_hbm, wuv_v, s_wuv, 64, D), (wo_hbm, wo_v, s_wo, 16, M)]
            wmb = [(wm_hbm.at[:, :, pl.ds(2 * M, 4 * M)], wmb_v, s_wmb, 8, 2 * M)]
            w1 = [(w1_hbm, w1_v, s_w1, 8, FH)]
            w2 = [([(w2_hbm, w2_v, fsems.at[i], 16, M)], O2[i] // 16, O2[i + 1] // 16) for i in range(N2)]
            kv = [(ckv_hbm.at[b], ckv_v.at[b], ksems.at[b], 16, Dc) for b in range(B)]
            kva, kvb = kv[:B // 2], kv[B // 2:]

            pltpu.make_async_copy(c_hbm, c_v, s_c).start()
            pltpu.make_async_copy(x_hbm, x_v, s_x).start()
            _stream(wma, 0, 16)
            _stream(wqk, 0, 64)

            _wait(c_v, s_c)
            cc = c_v[...].astype(_F32)
            sc = (cc * jax.nn.sigmoid(cc)).astype(_BF16)
            _wait(wma_v, s_wma)
            moda = jnp.dot(sc, _rows(wma_v), preferred_element_type=_F32)
            _wait(x_v, s_x)
            x = x_v[...].astype(_F32)
            h = (_layernorm(x) * (1.0 + moda[:, M:]) + moda[:, :M]).astype(_BF16)

            _stream(kva, 0, 16)
            _wait(wq_v, s_wq)
            _split_heads(wq_v, w32_v, tmp_v)
            _stream(kva, 16, 24)
            qs = []
            for j in range(HP):
                for w in _head_pair(tmp_v, j):
                    q = jnp.dot(h, w, preferred_element_type=_F32)
                    qs.append((q * D ** -0.5).astype(_BF16))
            _stream(kva, 24, 32)
            _wait(wuk_v, s_wuk)
            _split_heads(wuk_v, w32_v, tmp_v)
            _stream(kva, 32, 40)
            for j in range(HP):
                for s, w in enumerate(_head_pair(tmp_v, j)):
                    qa = jax.lax.dot_general(qs[2 * j + s], w, _NT, preferred_element_type=_F32)
                    for n in range(NC):
                        qa_v[n, pl.ds(2 * j + s, B, stride=H), :] = qa[:, n * 128:(n + 1) * 128]
            _stream(kva, 40, 64)
            _stream(kvb, 0, 16)

            ahead = [(0, kvb, 16, 32), (1, kvb, 32, 48), (2, kvb, 48, 64),
                     (3, wvo, 0, 26), (4, wvo, 26, 42), (5, wvo, 42, 58), (6, wvo, 58, 64),
                     (6, wmb, 0, 10)]

            def attend(b, carry):
                _wait(ckv_v.at[b], ksems.at[b])
                row = pl.ds(pl.multiple_of(b * H, H), H)
                qa = jnp.concatenate([qa_v[n, row, :] for n in range(NC)], axis=1).astype(_BF16)
                s = jax.lax.dot_general(qa, _rows(ckv_v.at[b]), _NT, preferred_element_type=_F32)
                p = jnp.exp(s - jnp.max(s, axis=-1, keepdims=True))
                l = jnp.sum(p, axis=-1, keepdims=True)
                o = jnp.dot(p.astype(_BF16), _rows(ckv_v.at[b]), preferred_element_type=_F32) / l
                for n in range(NC):
                    oc_v[n, row, :] = o[:, n * 128:(n + 1) * 128]

                for k, *request in ahead:
                    pl.when(b == k)(functools.partial(_stream, *request))
                return carry

            jax.lax.fori_loop(0, B, attend, 0)

            _stream(wmb, 10, 16)
            _stream(w1, 0, 24)
            _wait(wuv_v, s_wuv)
            _split_heads(wuv_v, w32_v, tmp_v)
            _stream(w1, 24, 32)
            _stream(*w2[0])
            ctx = []
            for j in range(HP):
                for s, w in enumerate(_head_pair(tmp_v, j)):
                    oc = jnp.concatenate(
                        [oc_v[n, pl.ds(2 * j + s, B, stride=H), :] for n in range(NC)], axis=1)
                    ctx.append(jnp.dot(oc.astype(_BF16), w, preferred_element_type=_F32).astype(_BF16))
            for request in w2[1:]:
                _stream(*request)
            _wait(wo_v, s_wo)
            att = jnp.dot(jnp.concatenate(ctx, axis=1), _rows(wo_v), preferred_element_type=_F32)
            _wait(wmb_v, s_wmb)
            modb = jnp.dot(sc, _rows(wmb_v), preferred_element_type=_F32)
            x1 = x + modb[:, :M] * att
            h2 = (_layernorm(x1) * (1.0 + modb[:, 2 * M:3 * M]) + modb[:, M:2 * M]).astype(_BF16)

            _wait(w1_v, s_w1)
            a = jnp.maximum(jnp.dot(h2, _rows(w1_v), preferred_element_type=_F32), 0.0).astype(_BF16)
            y = jnp.zeros((B, M), _F32)
            for i in range(N2):
                chunk = w2_v.at[:, pl.ds(O2[i], W2[i])]
                a_i = jnp.concatenate([a[:, O2[i]:O2[i + 1]], a[:, FH + O2[i]:FH + O2[i + 1]]], axis=1)
                _wait(chunk, fsems.at[i])
                y += jnp.dot(a_i, _rows(chunk), preferred_element_type=_F32)
            o_ref[...] = (x1 + modb[:, 3 * M:] * y).astype(o_ref.dtype)

        pl.run_scoped(main, pltpu.SemaphoreType.DMA((9,)), pltpu.SemaphoreType.DMA((B,)),
                      pltpu.SemaphoreType.DMA((N2,)))

    scratch = [
        pltpu.VMEM((B, M), _BF16),
        pltpu.VMEM((B, M), _BF16),
        pltpu.VMEM((B, _S, Sk // _S, Dc), _BF16),
        pltpu.VMEM((_S, M * H // _S, D), _BF16),
        pltpu.VMEM((_S, Dc * H // _S, D), _BF16),
        pltpu.VMEM((_S, Dc * H // _S, D), _BF16),
        pltpu.VMEM((_S, H * D // _S, M), _BF16),
        pltpu.VMEM((2, M // 2, F), _BF16),
        pltpu.VMEM((2, FH, M), _BF16),
        pltpu.VMEM((_S, M // _S, 2 * M), _BF16),
        pltpu.VMEM((_S, M // _S, 4 * M), _BF16),
        pltpu.VMEM((_S, Dc * HP // _S, D), jnp.uint32),
        pltpu.VMEM((4, _S, Dc * HP // _S // 4, D), jnp.uint32),
        pltpu.VMEM((NC, B * H, 128), _F32),
        pltpu.VMEM((NC, B * H, 128), _F32),
    ]
    return kernel, scratch


@jax.jit
def pallas_adaLN_cond__compressed_kv_cla__dense_activation_relu__decode_kernel(
    A_x: jax.Array,
    A_c_kv: jax.Array,
    A_w_q: jax.Array,
    A_w_uk: jax.Array,
    A_w_uv: jax.Array,
    A_w_o: jax.Array,
    B_x: jax.Array,
    B_w1: jax.Array,
    B_w2: jax.Array,
    c: jax.Array,
    w_mod: jax.Array,
):
    del B_x
    B, Sq, M = A_x.shape
    _, Sk, Dc = A_c_kv.shape
    _, H, D = A_w_q.shape
    F = B_w1.shape[1]
    assert Sq == 1
    kernel, scratch = _build(B, H, Sk, D, M, Dc, F)
    out = pl.pallas_call(
        kernel,
        out_shape=jax.ShapeDtypeStruct((B, M), A_x.dtype),
        in_specs=[pl.BlockSpec(memory_space=pl.ANY)] * 10,
        scratch_shapes=scratch,
        compiler_params=pltpu.CompilerParams(vmem_limit_bytes=100 * 1024 * 1024),
    )(A_x.reshape(B, M), A_c_kv.reshape(B, _S, Sk // _S, Dc), A_w_q.reshape(_S, -1, D),
      A_w_uk.reshape(_S, -1, D), A_w_uv.reshape(_S, -1, D), A_w_o.reshape(_S, -1, M),
      B_w1.reshape(2, -1, F), B_w2.reshape(2, -1, M), c, w_mod.reshape(_S, -1, 6 * M))
    return out.reshape(B, Sq, M)
```
